```python
import jax
import jax.numpy as jnp

def _softmax(x, axis=-1):
    return jax.nn.softmax(x, axis=axis)

def _gelu(x):
    return jax.nn.gelu(x, approximate=True)

def _silu(x):
    return jax.nn.silu(x)

def _sigmoid(x):
    return jax.nn.sigmoid(x)

def _layernorm(x, axis=-1, eps=1e-05):
    m = jnp.mean(x, axis=axis, keepdims=True)
    v = jnp.var(x, axis=axis, keepdims=True)
    return (x - m) / jnp.sqrt(v + eps)

def _scatter_add(tgt, idx, src, axis=0):
    return tgt.at[idx].add(src)

def _segment_sum(src, seg, n):
    return jax.ops.segment_sum(src, seg, n)

class _Rng:

    def __init__(self, key):
        self._k = key

    def _next(self):
        self._k, sub = jax.random.split(self._k)
        return sub

    def normal(self, shape):
        return jax.random.normal(self._next(), shape, dtype=jnp.bfloat16)

    def randint(self, lo, hi, shape):
        return jax.random.randint(self._next(), shape, lo, hi, dtype=jnp.int32)

    def uniform(self, shape, lo=0.0, hi=1.0):
        return jax.random.uniform(self._next(), shape, jnp.bfloat16, lo, hi)

    def permutation(self, n):
        return jax.random.permutation(self._next(), n)
kernel_name = 'interleave_layers__memory_aug_recurrent_mem_tr__spectral_gfnet__prompt'

def setup_inputs():
    _rng = _Rng(jax.random.key(int.from_bytes(__import__("os").urandom(4), "little")))
    _w = lambda a: (lambda t: t.astype(jnp.bfloat16) if jnp.issubdtype(t.dtype, jnp.floating) else t)(jnp.asarray(a))

    def _A_setup():
        B, S, Dm = (1, 2048, 640)
        H, Dh = (32, 128)
        M, seg = (8, 32)
        seg = min(seg, S)
        S = S // seg * seg
        return {'x': _w((lambda *s: _rng.normal(s) * 0.05)(B, S, Dm)), 'mem0': _w((lambda *s: _rng.normal(s) * 0.05)(B, M, Dm)), 'Wq': _w((lambda *s: _rng.normal(s) * 0.05)(Dm, H, Dh) * Dm ** (-0.5)), 'Wk': _w((lambda *s: _rng.normal(s) * 0.05)(Dm, H, Dh) * Dm ** (-0.5)), 'Wv': _w((lambda *s: _rng.normal(s) * 0.05)(Dm, H, Dh) * Dm ** (-0.5)), 'Wo': _w((lambda *s: _rng.normal(s) * 0.05)(H, Dh, Dm) * (H * Dh) ** (-0.5)), 'seg_len': seg}
    _A_in = _A_setup()

    def _B_setup():
        B, S, D = (1, 2048, 640)
        Df = D // 2 + 1
        return {'x': _w((lambda *s: _rng.normal(s) * 0.05)(B, S, D)), 'w_r': _w((lambda *s: _rng.normal(s) * 0.05)(S, Df) * 0.02), 'w_i': _w((lambda *s: _rng.normal(s) * 0.05)(S, Df) * 0.02)}
    _B_in = _B_setup()
    return {'A_x': _A_in['x'], 'A_mem0': _A_in['mem0'], 'A_Wq': _A_in['Wq'], 'A_Wk': _A_in['Wk'], 'A_Wv': _A_in['Wv'], 'A_Wo': _A_in['Wo'], 'A_seg_len': _A_in['seg_len'], 'B_x': _B_in['x'], 'B_w_r': _B_in['w_r'], 'B_w_i': _B_in['w_i']}

def reference(A_x, A_mem0, A_Wq, A_Wk, A_Wv, A_Wo, A_seg_len, B_x, B_w_r, B_w_i):

    def _A_ref(x, mem0, Wq, Wk, Wv, Wo, seg_len):
        B, S, Dm = x.shape
        H, Dh = (Wq.shape[1], Wq.shape[2])
        M = mem0.shape[1]
        scale = Dh ** (-0.5)
        n_seg = S // seg_len
        L = M + seg_len
        idx = jnp.arange(L)
        mask = (idx[:, None] < M) | (idx[:, None] >= idx[None, :])
        mem = mem0
        outs = []
        for s in range(n_seg):
            xs = x[:, s * seg_len:(s + 1) * seg_len, :].copy()
            h = jnp.concatenate([mem, xs], axis=1)
            q = jnp.einsum('btd,dhe->bhte', h, Wq)
            k = jnp.einsum('btd,dhe->bhte', h, Wk)
            v = jnp.einsum('btd,dhe->bhte', h, Wv)
            scores = jnp.einsum('bhqe,bhke->bhqk', q, k) * scale
            scores = jnp.where(mask[None, None], scores, -1000000000.0)
            p = _softmax(scores, axis=-1)
            o = jnp.einsum('bhqk,bhke->bhqe', p, v)
            o = jnp.einsum('bhte,hed->btd', o, Wo)
            mem = o[:, :M, :].copy()
            outs.append(o[:, M:, :])
        return jnp.concatenate(outs, axis=1)

    def _B_ref(x, w_r, w_i):
        B, S, D = x.shape
        X = (lambda x, axes=(-2, -1): jnp.fft.rfft2(x.astype(jnp.float32), axes=axes))(x, axes=(-2, -1))
        W = w_r + 1j * w_i
        X = X * W
        y = (lambda x, s, axes=(-2, -1): jnp.fft.irfft2(x, s=s, axes=axes).astype(jnp.bfloat16))(X, (S, D), axes=(-2, -1))
        return y
    x = A_x
    x = x + _A_ref(_layernorm(x, axis=-1), A_mem0, A_Wq, A_Wk, A_Wv, A_Wo, A_seg_len)
    x = x + _B_ref(_layernorm(x, axis=-1), B_w_r, B_w_i)
    x = x + _A_ref(_layernorm(x, axis=-1), A_mem0, A_Wq, A_Wk, A_Wv, A_Wo, A_seg_len)
    x = x + _B_ref(_layernorm(x, axis=-1), B_w_r, B_w_i)
    return x
```

```python
import functools

import numpy as np
import jax
import jax.numpy as jnp
import jax.experimental.pallas as pl
import jax.experimental.pallas.tpu as pltpu

F32 = jnp.float32
BF16 = jnp.bfloat16
U32 = jnp.uint32

S, D, H, DH, M, SEG = 2048, 640, 32, 128, 8, 32
L = M + SEG
NSEG = S // SEG
NT = D // 128
DF = D // 2 + 1
FP = 384
NF = FP // 128
N1, N2 = 64, 32
NP = H // 2
LOG2E = 1.4426950408889634
WCH = 5


def _consts():
    d = np.arange(D)[:, None]
    f = np.arange(FP)[None, :]
    th = 2.0 * np.pi * ((d * f) % D) / D
    c = np.where(f < DF, np.cos(th), 0.0)
    s = np.where((f < DF - 1) & (f > 0), -np.sin(th), 0.0)
    fd = np.concatenate([c, s], axis=1)

    k1 = np.arange(N1)[None, :, None]
    n1 = np.arange(N1)[None, None, :]
    n2 = np.arange(N2)[:, None, None]
    th = 2.0 * np.pi * (((N2 * n1 + n2) * k1) % S) / S
    c, s = np.cos(th), np.sin(th)
    m1 = np.concatenate([np.concatenate([c, s], 2), np.concatenate([-s, c], 2)], 1)

    k2 = np.arange(N2)[:, None]
    n2 = np.arange(N2)[None, :]
    th = 2.0 * np.pi * ((k2 * n2) % N2) / N2
    c, s = np.cos(th), np.sin(th)
    m2 = np.kron(np.eye(2), np.block([[c, s], [-s, c]]))

    cf = np.where((f == 0) | (f == DF - 1), 1.0, 2.0) * (f < DF) / (S * D)
    as_bf = lambda a: np.ascontiguousarray(a).astype(np.float32).astype(BF16)
    return (as_bf(fd), as_bf(fd.T), as_bf(m1), as_bf(m1.transpose(0, 2, 1)),
            as_bf(m2), as_bf(m2.T), cf.astype(np.float32))


def _dot(a, b):
    return jax.lax.dot_general(a, b, (((1,), (0,)), ((), ())), preferred_element_type=F32)


def _dot_nt(a, b):
    return jax.lax.dot_general(a, b, (((1,), (1,)), ((), ())), preferred_element_type=F32)


def _ln(x):
    m = jnp.mean(x, axis=-1, keepdims=True)
    xc = x - m
    v = jnp.mean(xc * xc, axis=-1, keepdims=True)
    return xc * jax.lax.rsqrt(v + 1e-5)


def _rnd(x):
    return x.astype(BF16).astype(F32)


def _ld(ref, rows):
    return jnp.concatenate([ref[t, rows, :] for t in range(ref.shape[0])], axis=1)


def _st(ref, rows, val):
    for t in range(ref.shape[0]):
        ref[t, rows, :] = val[:, t * 128:(t + 1) * 128]


def _kernel(x_ref, mem0_ref, wq_hbm, wk_hbm, wv_hbm, wo_hbm, wr_ref, wi_ref,
            fd_ref, fdt_ref, m1_ref, m1t_ref, m2_ref, m2t_ref, cf_ref,
            out_ref,
            wraw, wqkv, wo32, xs, hz, obuf, bufa, wpad, wnat, sems):
    rows = D * NP // WCH
    copies = []
    for c in range(WCH):
        for i, w in enumerate((wq_hbm, wk_hbm, wv_hbm)):
            cp = pltpu.make_async_copy(w.bitcast(U32).at[pl.ds(c * rows, rows)],
                                       wraw.at[i, pl.ds(c * rows, rows)],
                                       sems.at[c * 3 + i])
            cp.start()
            copies.append(cp)
    wo_cp = pltpu.make_async_copy(wo_hbm.bitcast(U32), wo32, sems.at[3 * WCH])
    wo_cp.start()

    def prep(i, _):
        r = pl.ds(pl.multiple_of(i * 64, 64), 64)
        x = x_ref[r, :].astype(F32)
        _st(xs, r, x)
        _st(hz, r, _ln(x))
    jax.lax.fori_loop(0, S // 64, prep, None)

    for i, w in enumerate((wr_ref, wi_ref)):
        wpad[pl.ds(DF - 1, FP - DF + 1), :] = jnp.zeros((FP - DF + 1, S), F32)
        wpad[pl.ds(0, DF), :] = w[...].astype(F32)
        for t in range(NF):
            for c in range(S // 512):
                blk = wpad[t * 128:(t + 1) * 128, c * 512:(c + 1) * 512].T
                wnat[i, t, c * 512:(c + 1) * 512, :] = blk * cf_ref[:, t * 128:(t + 1) * 128]

    dch = D // WCH
    for c in range(WCH):
        for i in range(3):
            copies[c * 3 + i].wait()

            def regroup(j, _, c=c, i=i):
                base = c * dch * NP + j
                a = wraw[i, pl.ds(base, dch // 2, stride=2 * NP), :]
                b = wraw[i, pl.ds(base + NP, dch // 2, stride=2 * NP), :]
                r = pl.ds(c * dch // 2, dch // 2)
                wqkv[j, r, pl.ds(i * 256, 128)] = (a & 0xFFFF) | (b << 16)
                wqkv[j, r, pl.ds(i * 256 + 128, 128)] = (a >> 16) | (b & np.uint32(0xFFFF0000))
            jax.lax.fori_loop(0, NP, regroup, None)
    wo_cp.wait()

    ri = jax.lax.broadcasted_iota(jnp.int32, (2 * L, 2 * L), 0)
    ci = jax.lax.broadcasted_iota(jnp.int32, (2 * L, 2 * L), 1)
    same = (ri < L) == (ci < L)
    rl = jnp.where(ri < L, ri, ri - L)
    cl = jnp.where(ci < L, ci, ci - L)
    keep = same & ((rl < M) | (rl >= cl))
    fill = jnp.where(same, -1e9 * LOG2E, -jnp.inf).astype(F32)

    def layer(_, carry):
        def seg(s, mem):
            r = pl.ds(pl.multiple_of(s * SEG, SEG), SEG)
            h = jnp.concatenate([mem, _ld(hz, r)], axis=0)
            for j in range(NP):
                qkv = _dot(h, pltpu.bitcast(wqkv[j], BF16))
                q, k, v = (jnp.concatenate([qkv[:, o:o + 128], qkv[:, o + 128:o + 256]], axis=0)
                           for o in (0, 256, 512))
                t = _dot_nt(q, k.astype(BF16)) * (DH ** -0.5 * LOG2E)
                t = jnp.where(keep, t, fill)
                e = jnp.exp2(t - jnp.max(t, axis=-1, keepdims=True))
                o = _dot(e, v.astype(BF16)) / jnp.sum(e, axis=-1, keepdims=True)
                obuf[:, j * 256:j * 256 + 128] = o[:L]
                obuf[:, j * 256 + 128:(j + 1) * 256] = o[L:]
            y = _dot(obuf[...], pltpu.bitcast(wo32[...], BF16))
            x = _rnd(_ld(xs, r) + y[M:])
            _st(xs, r, x)
            _st(hz, r, _ln(x))
            return y[:M]
        jax.lax.fori_loop(0, NSEG, seg, mem0_ref[...].astype(F32))

        def fwd(n2, _):
            z = _ld(hz, pl.ds(n2, N1, stride=N2)).astype(BF16)
            zf = _dot(z, fd_ref[...]).astype(BF16)
            a = _dot(m1_ref[n2], jnp.concatenate([zf[:, :FP], zf[:, FP:]], axis=0))
            _st(bufa, pl.ds(n2, N1, stride=2 * N2), a[:N1])
            _st(bufa, pl.ds(n2 + N2, N1, stride=2 * N2), a[N1:])
        jax.lax.fori_loop(0, N2, fwd, None)

        def mid(p, _):
            r = pl.ds(pl.multiple_of(p * 128, 128), 128)
            xf = _dot(m2_ref[...], _ld(bufa, r).astype(BF16))
            ys = []
            for u in range(2):
                kr = pl.ds(2 * p + u, N2, stride=N1)
                wr, wi = _ld(wnat.at[0], kr), _ld(wnat.at[1], kr)
                xr, xi = xf[u * 64:u * 64 + 32], xf[u * 64 + 32:u * 64 + 64]
                ys += [xr * wr - xi * wi, xr * wi + xi * wr]
            _st(bufa, r, _dot(m2t_ref[...], jnp.concatenate(ys, axis=0).astype(BF16)))
        jax.lax.fori_loop(0, N1 // 2, mid, None)

        def inv(n2, _):
            b = jnp.concatenate([_ld(bufa, pl.ds(n2, N1, stride=2 * N2)),
                                 _ld(bufa, pl.ds(n2 + N2, N1, stride=2 * N2))], axis=0)
            yf = _dot(m1t_ref[n2], b.astype(BF16)).astype(BF16)
            y = _dot(jnp.concatenate([yf[:N1], yf[N1:]], axis=1), fdt_ref[...])
            r = pl.ds(n2, N1, stride=N2)
            x = _rnd(_ld(xs, r) + y)
            _st(xs, r, x)
            _st(hz, r, _ln(x))
        jax.lax.fori_loop(0, N2, inv, None)
        return carry
    jax.lax.fori_loop(0, 2, layer, 0)

    def fin(i, _):
        r = pl.ds(pl.multiple_of(i * 128, 128), 128)
        out_ref[r, :] = _ld(xs, r).astype(BF16)
    jax.lax.fori_loop(0, S // 128, fin, None)


@functools.partial(jax.jit, static_argnames=("A_seg_len",))
def pallas_interleave_layers__memory_aug_recurrent_mem_tr__spectral_gfnet__prompt_kernel(
    A_x, A_mem0, A_Wq, A_Wk, A_Wv, A_Wo, A_seg_len, B_x, B_w_r, B_w_i,
):
    del B_x
    assert A_seg_len == SEG and A_x.shape == (1, S, D) and A_Wq.shape == (D, H, DH)
    vmem = pl.BlockSpec(memory_space=pltpu.VMEM)
    hbm = pl.BlockSpec(memory_space=pl.ANY)
    consts = _consts()
    out = pl.pallas_call(
        _kernel,
        out_shape=jax.ShapeDtypeStruct((S, D), BF16),
        in_specs=[vmem, vmem, hbm, hbm, hbm, hbm, vmem, vmem] + [vmem] * len(consts),
        out_specs=vmem,
        scratch_shapes=[
            pltpu.VMEM((3, D * NP + 64, DH), U32),
            pltpu.VMEM((NP, D // 2, 768), U32),
            pltpu.VMEM((H * DH // 2, D), U32),
            pltpu.VMEM((NT, S + 64, 128), F32),
            pltpu.VMEM((NT, S + 64, 128), F32),
            pltpu.VMEM((L, H * DH), F32),
            pltpu.VMEM((NF, 2 * S + 64, 128), F32),
            pltpu.VMEM((FP, S), F32),
            pltpu.VMEM((2, NF, S + 64, 128), F32),
            pltpu.SemaphoreType.DMA((3 * WCH + 1,)),
        ],
        compiler_params=pltpu.CompilerParams(vmem_limit_bytes=110 * 1024 * 1024),
    )(A_x.reshape(S, D), A_mem0.reshape(M, D),
      A_Wq.reshape(D * H, DH), A_Wk.reshape(D * H, DH), A_Wv.reshape(D * H, DH),
      A_Wo.reshape(H * DH, D), B_w_r.T, B_w_i.T, *consts)
    return out.reshape(1, S, D)
```

```python
import functools

import numpy as np
import jax
import jax.numpy as jnp
import jax.experimental.pallas as pl
import jax.experimental.pallas.tpu as pltpu

F32 = jnp.float32
BF16 = jnp.bfloat16
U32 = jnp.uint32

S, D, H, DH, M, SEG = 2048, 640, 32, 128, 8, 32
L = M + SEG
NSEG = S // SEG
NT = D // 128
DF = D // 2 + 1
FP = 384
NF = FP // 128
N1, N2 = 64, 32
NP = H // 2
LOG2E = 1.4426950408889634
PX = SEG + 4
PA = 2 * N2 + 4
C1, C2 = float(np.cos(0.4 * np.pi)), float(np.cos(0.8 * np.pi))
S1, S2 = float(np.sin(0.4 * np.pi)), float(np.sin(0.8 * np.pi))
WCH = 5


def _consts():
    a = np.arange(128)[:, None]
    m = np.arange(64)
    f0 = np.concatenate([5 * np.arange(65), np.full(63, -1)])
    fs = [f0, np.concatenate([1 + 5 * m, 4 + 5 * m]), np.concatenate([2 + 5 * m, 3 + 5 * m])]
    g = []
    for r, f in enumerate(fs):
        f = f[None, :]
        th = 2.0 * np.pi * ((a * f) % D) / D
        c, s = np.cos(th), np.sin(th)
        if r == 0:
            g.append(np.concatenate([c * (f >= 0), -s * ((f > 0) & (f < DF - 1))], axis=1))
        else:
            sg = np.where(f % 5 == r, 1.0, -1.0)
            g.append(np.block([[c, -s], [sg * s, sg * c]]))
    f = np.concatenate(fs)[None, :]

    k1 = np.arange(N1)[None, :, None]
    n1 = np.arange(N1)[None, None, :]
    n2 = np.arange(N2)[:, None, None]
    th = 2.0 * np.pi * (((N2 * n1 + n2) * k1) % S) / S
    c, s = np.cos(th), np.sin(th)
    m1 = np.concatenate([np.concatenate([c, s], 2), np.concatenate([-s, c], 2)], 1)

    k2 = np.arange(N2)[:, None]
    n2 = np.arange(N2)[None, :]
    th = 2.0 * np.pi * ((k2 * n2) % N2) / N2
    c, s = np.cos(th), np.sin(th)
    m2 = np.kron(np.eye(2), np.block([[c, s], [-s, c]]))

    cf = np.where((f == 0) | (f == DF - 1), 1.0, 2.0) * (f >= 0) / (S * D)
    as_bf = lambda a: np.ascontiguousarray(a).astype(np.float32).astype(BF16)
    return (as_bf(g[0]), as_bf(g[0].T), as_bf(np.stack(g[1:])),
            as_bf(np.stack([x.T for x in g[1:]])), as_bf(m1), as_bf(m1.transpose(0, 2, 1)),
            as_bf(m2), as_bf(m2.T), cf.astype(np.float32))


def _dot(a, b):
    return jax.lax.dot_general(a, b, (((1,), (0,)), ((), ())), preferred_element_type=F32)


def _dot_nt(a, b):
    return jax.lax.dot_general(a, b, (((1,), (1,)), ((), ())), preferred_element_type=F32)


def _ln(x):
    m = jnp.mean(x, axis=-1, keepdims=True)
    xc = x - m
    v = jnp.mean(xc * xc, axis=-1, keepdims=True)
    return xc * jax.lax.rsqrt(v + 1e-5)


def _rnd(x):
    return x.astype(BF16).astype(F32)


def _ld(ref, rows):
    return jnp.concatenate([ref[t, rows, :] for t in range(ref.shape[0])], axis=1)


def _st(ref, rows, val):
    for t in range(ref.shape[0]):
        ref[t, rows, :] = val[:, t * 128:(t + 1) * 128]


def _kernel(x_ref, mem0_ref, wq_hbm, wk_hbm, wv_hbm, wo_hbm, wr_ref, wi_ref,
            g0_ref, g0t_ref, g_ref, gt_ref, m1_ref, m1t_ref, m2_ref, m2t_ref, cf_ref,
            out_ref,
            wraw, wqkv, wo32, xs, hz, obuf, bufa, bufb, wpad, wnat, sems):
    rows = D * NP // WCH
    copies = []
    for c in range(WCH):
        for i, w in enumerate((wq_hbm, wk_hbm, wv_hbm)):
            cp = pltpu.make_async_copy(w.bitcast(U32).at[pl.ds(c * rows, rows)],
                                       wraw.at[i, pl.ds(c * rows, rows)],
                                       sems.at[c * 3 + i])
            cp.start()
            copies.append(cp)
    wo_cp = pltpu.make_async_copy(wo_hbm.bitcast(U32), wo32, sems.at[3 * WCH])
    wo_cp.start()

    def prep(i, _):
        for u in range(4):
            x = x_ref[pl.ds(pl.multiple_of((4 * i + u) * SEG, SEG), SEG), :].astype(F32)
            r = pl.ds((4 * i + u) * PX, SEG)
            _st(xs, r, x)
            _st(hz, r, _ln(x))
    jax.lax.fori_loop(0, NSEG // 4, prep, None)

    for i, w in enumerate((wr_ref, wi_ref)):
        for c in range(S // 128):
            wpad[c, pl.ds(DF - 1, 8), :] = jnp.zeros((8, 128), F32)
            wpad[c, pl.ds(0, DF), :] = w[:, c * 128:(c + 1) * 128].astype(F32)
        for c in range(S // 128):
            res = lambda r: wpad[c, pl.ds(r, 64, stride=5), :]
            top = jnp.concatenate([wpad[c, pl.ds(DF - 1, 8), :], jnp.zeros((56, 128), F32)], axis=0)
            for t, (lo, hi) in enumerate(((res(0), top), (res(1), res(4)), (res(2), res(3)))):
                blk = jnp.concatenate([lo, hi], axis=0).T * cf_ref[:, t * 128:(t + 1) * 128]
                wnat[i, t, pl.ds(2 * c * PA, N1), :] = blk[:N1]
                wnat[i, t, pl.ds((2 * c + 1) * PA, N1), :] = blk[N1:]

    dch = D // WCH
    for c in range(WCH):
        for i in range(3):
            copies[c * 3 + i].wait()

            def regroup(j, _, c=c, i=i):
                base = c * dch * NP + j
                a = wraw[i, pl.ds(base, dch // 2, stride=2 * NP), :]
                b = wraw[i, pl.ds(base + NP, dch // 2, stride=2 * NP), :]
                r = pl.ds(c * dch // 2, dch // 2)
                wqkv[j, r, pl.ds(i * 256, 128)] = (a & 0xFFFF) | (b << 16)
                wqkv[j, r, pl.ds(i * 256 + 128, 128)] = (a >> 16) | (b & np.uint32(0xFFFF0000))
            jax.lax.fori_loop(0, NP, regroup, None)
    wo_cp.wait()

    ri = jax.lax.broadcasted_iota(jnp.int32, (2 * L, 2 * L), 0)
    ci = jax.lax.broadcasted_iota(jnp.int32, (2 * L, 2 * L), 1)
    same = (ri < L) == (ci < L)
    rl = jnp.where(ri < L, ri, ri - L)
    cl = jnp.where(ci < L, ci, ci - L)
    keep = same & ((rl < M) | (rl >= cl))
    fill = jnp.where(same, -1e9 * LOG2E, -jnp.inf).astype(F32)

    def layer(_, carry):
        def seg(s, mem):
            r = pl.ds(s * PX, SEG)
            h = jnp.concatenate([mem, _ld(hz, r)], axis=0)
            st = {}

            def stack(a, o):
                return jnp.concatenate([a[:, o:o + 128], a[:, o + 128:o + 256]], axis=0)

            def proj_qk(j):
                a = _dot(h, pltpu.bitcast(wqkv[j, :, 0:512], BF16))
                st["q", j], st["k", j] = stack(a, 0), stack(a, 256).astype(BF16)

            def proj_v(j):
                st["v", j] = stack(_dot(h, pltpu.bitcast(wqkv[j, :, 512:768], BF16)), 0).astype(BF16)

            def scores(j):
                t = _dot_nt(st.pop(("q", j)), st.pop(("k", j))) * (DH ** -0.5 * LOG2E)
                t = jnp.where(keep, t, fill)
                st["e", j] = jnp.exp2(t - jnp.max(t, axis=-1, keepdims=True))

            def pv(j):
                e = st.pop(("e", j))
                o = _dot(e, st.pop(("v", j))) / jnp.sum(e, axis=-1, keepdims=True)
                obuf[:, j * 256:j * 256 + 128] = o[:L]
                obuf[:, j * 256 + 128:(j + 1) * 256] = o[L:]

            def proj_o(a, b):
                return _dot(obuf[:, a * 256:b * 256], pltpu.bitcast(wo32[a * 128:b * 128, :], BF16))

            proj_qk(0)
            for j in range(NP):
                if j + 1 < NP:
                    proj_qk(j + 1)
                else:
                    y = proj_o(0, 4)
                scores(j)
                proj_v(j)
                if j > 0:
                    pv(j - 1)
            y += proj_o(4, 8)
            pv(NP - 1)
            y += proj_o(8, NP)
            x = _rnd(_ld(xs, r) + y[M:])
            _st(xs, r, x)
            _st(hz, r, _ln(x))
            return y[:M]
        jax.lax.fori_loop(0, NSEG, seg, mem0_ref[...].astype(F32))

        def skew(n, first, second):
            prev = first(0)
            for u in range(n):
                nxt = first(u + 1) if u + 1 < n else None
                second(u, prev)
                prev = nxt

        tile = lambda a, t: a[:, t * 128:(t + 1) * 128]
        UN = 8

        def fwd(i, _):
            def feat(u):
                r = pl.ds(i * UN + u, N1, stride=PX)
                z0, z1, z2, z3, z4 = (hz[t, r, :] for t in range(NT))
                s1, d1, s2, d2 = z1 + z4, z1 - z4, z2 + z3, z2 - z3
                u1 = jnp.concatenate([z0 + C1 * s1 + C2 * s2, -S1 * d1 - S2 * d2], axis=1)
                u2 = jnp.concatenate([z0 + C2 * s1 + C1 * s2, S1 * d2 - S2 * d1], axis=1)
                xf = [_dot(z0 + s1 + s2, g0_ref[...]), _dot(u1, g_ref[0]), _dot(u2, g_ref[1])]
                return jnp.concatenate(
                    [jnp.concatenate([tile(a, c) for a in xf], axis=1) for c in range(2)],
                    axis=0).astype(BF16)

            def seq(u, zf):
                n2 = i * UN + u
                a = _dot(m1_ref[n2], zf)
                _st(bufa, pl.ds(n2, N1, stride=PA), a[:N1])
                _st(bufa, pl.ds(n2 + N2, N1, stride=PA), a[N1:])
            skew(UN, feat, seq)
        jax.lax.fori_loop(0, N2 // UN, fwd, None)

        def mid(i, _):
            rows = lambda u, w: pl.ds((2 * (i * UN + u) + w) * PA, 2 * N2)

            def f2(u):
                a = jnp.concatenate([_ld(bufa, rows(u, 0)), _ld(bufa, rows(u, 1))], axis=0)
                xf = _dot(m2_ref[...], a.astype(BF16))
                ys = []
                for w in range(2):
                    kr = pl.ds(2 * (i * UN + u) + w, N2, stride=PA)
                    wr, wi = _ld(wnat.at[0], kr), _ld(wnat.at[1], kr)
                    xr, xi = xf[w * 64:w * 64 + 32], xf[w * 64 + 32:w * 64 + 64]
                    ys += [xr * wr - xi * wi, xr * wi + xi * wr]
                return jnp.concatenate(ys, axis=0).astype(BF16)

            def i2(u, y):
                b = _dot(m2t_ref[...], y)
                _st(bufb, rows(u, 0), b[:64])
                _st(bufb, rows(u, 1), b[64:])
            skew(UN, f2, i2)
        jax.lax.fori_loop(0, N1 // 2 // UN, mid, None)

        def inv(i, _):
            def seq(u):
                n2 = i * UN + u
                b = jnp.concatenate([_ld(bufb, pl.ds(n2, N1, stride=PA)),
                                     _ld(bufb, pl.ds(n2 + N2, N1, stride=PA))], axis=0)
                return _dot(m1t_ref[n2], b.astype(BF16)).astype(BF16)

            def feat(u, yf):
                ri_ = lambda t: jnp.concatenate([tile(yf[:N1], t), tile(yf[N1:], t)], axis=1)
                v0 = _dot(ri_(0), g0t_ref[...])
                v1, v2 = _dot(ri_(1), gt_ref[0]), _dot(ri_(2), gt_ref[1])
                a1, b1, a2, b2 = tile(v1, 0), tile(v1, 1), tile(v2, 0), tile(v2, 1)
                s1, s2 = v0 + C1 * a1 + C2 * a2, v0 + C2 * a1 + C1 * a2
                d1, d2 = -S1 * b1 - S2 * b2, S1 * b2 - S2 * b1
                y = jnp.concatenate([v0 + a1 + a2, s1 + d1, s2 + d2, s2 - d2, s1 - d1], axis=1)
                r = pl.ds(i * UN + u, N1, stride=PX)
                x = _rnd(_ld(xs, r) + y)
                _st(xs, r, x)
                _st(hz, r, _ln(x))
            skew(UN, seq, feat)
        jax.lax.fori_loop(0, N2 // UN, inv, None)
        return carry
    jax.lax.fori_loop(0, 2, layer, 0)

    def fin(i, _):
        for u in range(4):
            r = pl.ds(pl.multiple_of((4 * i + u) * SEG, SEG), SEG)
            out_ref[r, :] = _ld(xs, pl.ds((4 * i + u) * PX, SEG)).astype(BF16)
    jax.lax.fori_loop(0, S // 128, fin, None)


@functools.partial(jax.jit, static_argnames=("A_seg_len",))
def pallas_interleave_layers__memory_aug_recurrent_mem_tr__spectral_gfnet__prompt_kernel(
    A_x, A_mem0, A_Wq, A_Wk, A_Wv, A_Wo, A_seg_len, B_x, B_w_r, B_w_i,
):
    del B_x
    assert A_seg_len == SEG and A_x.shape == (1, S, D) and A_Wq.shape == (D, H, DH)
    vmem = pl.BlockSpec(memory_space=pltpu.VMEM)
    hbm = pl.BlockSpec(memory_space=pl.ANY)
    consts = _consts()
    out = pl.pallas_call(
        _kernel,
        out_shape=jax.ShapeDtypeStruct((S, D), BF16),
        in_specs=[vmem, vmem, hbm, hbm, hbm, hbm, vmem, vmem] + [vmem] * len(consts),
        out_specs=vmem,
        scratch_shapes=[
            pltpu.VMEM((3, D * NP + 64, DH), U32),
            pltpu.VMEM((NP, D // 2, 768), U32),
            pltpu.VMEM((H * DH // 2, D), U32),
            pltpu.VMEM((NT, (NSEG + 2) * PX, 128), F32),
            pltpu.VMEM((NT, (NSEG + 2) * PX, 128), F32),
            pltpu.VMEM((L, H * DH), F32),
            pltpu.VMEM((NF, (N1 + 2) * PA, 128), F32),
            pltpu.VMEM((NF, (N1 + 2) * PA, 128), F32),
            pltpu.VMEM((S // 128, DF + 7, 128), F32),
            pltpu.VMEM((2, NF, (N2 + 2) * PA, 128), F32),
            pltpu.SemaphoreType.DMA((3 * WCH + 1,)),
        ],
        compiler_params=pltpu.CompilerParams(vmem_limit_bytes=110 * 1024 * 1024),
    )(A_x.reshape(S, D), A_mem0.reshape(M, D),
      A_Wq.reshape(D * H, DH), A_Wk.reshape(D * H, DH), A_Wv.reshape(D * H, DH),
      A_Wo.reshape(H * DH, D), B_w_r.T, B_w_i.T, *consts)
    return out.reshape(1, S, D)
```

```python
import functools

import numpy as np
import jax
import jax.numpy as jnp
import jax.experimental.pallas as pl
import jax.experimental.pallas.tpu as pltpu

F32 = jnp.float32
BF16 = jnp.bfloat16
U32 = jnp.uint32

S, D, H, DH, M, SEG = 2048, 640, 32, 128, 8, 32
L = M + SEG
NSEG = S // SEG
NT = D // 128
DF = D // 2 + 1
FP = 384
NF = FP // 128
N1, N2 = 64, 32
NP = H // 2
LAG_V, LAG_P, NG, G0, G1 = 2, 4, 2, 2, 6
USEG = 2
XHEAD = USEG + 1
UN = 8
NLATE = 11
LOG2E = 1.4426950408889634
PX = SEG + 4
PA = 2 * N2 + 4
C1, C2 = float(np.cos(0.4 * np.pi)), float(np.cos(0.8 * np.pi))
S1, S2 = float(np.sin(0.4 * np.pi)), float(np.sin(0.8 * np.pi))
WCH = 5


def _consts():
    a = np.arange(128)[:, None]
    m = np.arange(64)
    f0 = np.concatenate([5 * np.arange(65), np.full(63, -1)])
    fs = [f0, np.concatenate([1 + 5 * m, 4 + 5 * m]), np.concatenate([2 + 5 * m, 3 + 5 * m])]
    g = []
    for r, f in enumerate(fs):
        f = f[None, :]
        th = 2.0 * np.pi * ((a * f) % D) / D
        c, s = np.cos(th), np.sin(th)
        if r == 0:
            g.append(np.concatenate([c * (f >= 0), -s * ((f > 0) & (f < DF - 1))], axis=1))
        else:
            sg = np.where(f % 5 == r, 1.0, -1.0)
            g.append(np.block([[c, -s], [sg * s, sg * c]]))
    f = np.concatenate(fs)[None, :]

    k1 = np.arange(N1)[None, :, None]
    n1 = np.arange(N1)[None, None, :]
    n2 = np.arange(N2)[:, None, None]
    th = 2.0 * np.pi * (((N2 * n1 + n2) * k1) % S) / S
    c, s = np.cos(th), np.sin(th)
    m1 = np.concatenate([np.concatenate([c, s], 2), np.concatenate([-s, c], 2)], 1)

    k2 = np.arange(N2)[:, None]
    n2 = np.arange(N2)[None, :]
    th = 2.0 * np.pi * ((k2 * n2) % N2) / N2
    c, s = np.cos(th), np.sin(th)
    m2 = np.kron(np.eye(2), np.block([[c, s], [-s, c]]))

    cf = np.where((f == 0) | (f == DF - 1), 1.0, 2.0) * (f >= 0) / (S * D)
    as_bf = lambda a: np.ascontiguousarray(a).astype(np.float32).astype(BF16)
    return (as_bf(g[0]), as_bf(g[0].T), as_bf(np.stack(g[1:])),
            as_bf(np.stack([x.T for x in g[1:]])), as_bf(m1), as_bf(m1.transpose(0, 2, 1)),
            as_bf(m2), as_bf(m2.T), cf.astype(np.float32))


def _schedule():
    ops = [("qk", 0)]
    for j in range(NP + LAG_P):
        if j + 1 < NP:
            ops.append(("qk", j + 1))
        if j < NP:
            ops.append(("s", j))
        if 0 <= j - LAG_V < NP:
            ops.append(("v", j - LAG_V))
        if j - LAG_V == NP - 1:
            ops.append(("h",))
        if j - LAG_P == NP - NG:
            ops += [("o", 0, G0), ("gate", *range(NP - NG, NP)), ("o", G0, G1)]
        if j - LAG_P >= 0:
            ops.append(("pv", j - LAG_P))
    return ops + [("o", G1, NP)]


def _dot(a, b):
    return jax.lax.dot_general(a, b, (((1,), (0,)), ((), ())), preferred_element_type=F32)


def _dot_nt(a, b):
    return jax.lax.dot_general(a, b, (((1,), (1,)), ((), ())), preferred_element_type=F32)


def _ln(x):
    m = jnp.mean(x, axis=-1, keepdims=True)
    xc = x - m
    v = jnp.mean(xc * xc, axis=-1, keepdims=True)
    return xc * jax.lax.rsqrt(v + 1e-5)


def _rnd(x):
    return x.astype(BF16).astype(F32)


def _ld(ref, rows):
    return jnp.concatenate([ref[t, rows, :] for t in range(ref.shape[0])], axis=1)


def _st(ref, rows, val):
    for t in range(ref.shape[0]):
        ref[t, rows, :] = val[:, t * 128:(t + 1) * 128]


def _kernel(mem0_ref, x_hbm, wq_hbm, wk_hbm, wv_hbm, wo_hbm, *refs):
    late_hbm, out_hbm, late = refs[:NLATE], refs[NLATE], refs[NLATE + 1:2 * NLATE + 1]
    (xin, xout, wraw, wqkv, wo32, xs, hz, hbuf, gate, obuf, bufa, bufb, wpad, wnat,
     sems) = refs[2 * NLATE + 1:]
    wr_ref, wi_ref, g0_ref, g0t_ref, g_ref, gt_ref, m1_ref, m1t_ref, m2_ref, m2t_ref, cf_ref = late

    rows = D * NP // WCH
    pairs = [(x_hbm.at[pl.ds(0, XHEAD)], xin.at[pl.ds(0, XHEAD)]), (wo_hbm.bitcast(U32), wo32)]
    pairs += [(w.bitcast(U32).at[pl.ds(c * rows, rows)], wraw.at[i, pl.ds(c * rows, rows)])
              for c in range(WCH) for i, w in enumerate((wq_hbm, wk_hbm, wv_hbm))]
    tail = pl.ds(XHEAD, NSEG - XHEAD)
    pairs += [(x_hbm.at[tail], xin.at[tail])] + list(zip(late_hbm, late))
    loads = [pltpu.make_async_copy(a, b, sems.at[n]) for n, (a, b) in enumerate(pairs)]
    x_cp, wo_cp, copies = loads[0], loads[1], loads[2:2 + 3 * WCH]
    xt_cp, late_cp = loads[2 + 3 * WCH], loads[3 + 3 * WCH:]
    out_cp = [pltpu.make_async_copy(xout.at[i], out_hbm.at[:, i], sems.at[len(loads) + i])
              for i in range(N2 // UN)]
    for cp in loads[:2 + 3 * WCH]:
        cp.start()

    def filter_prep():
        for i, w in enumerate((wr_ref, wi_ref)):
            for c in range(S // 128):
                wpad[c, pl.ds(DF - 1, 8), :] = jnp.zeros((8, 128), F32)
                wpad[c, pl.ds(0, DF), :] = w[:, c * 128:(c + 1) * 128].astype(F32)
            for c in range(S // 128):
                res = lambda r: wpad[c, pl.ds(r, 64, stride=5), :]
                top = jnp.concatenate(
                    [wpad[c, pl.ds(DF - 1, 8), :], jnp.zeros((56, 128), F32)], axis=0)
                for t, (lo, hi) in enumerate(((res(0), top), (res(1), res(4)), (res(2), res(3)))):
                    blk = jnp.concatenate([lo, hi], axis=0).T * cf_ref[:, t * 128:(t + 1) * 128]
                    wnat[i, t, pl.ds(2 * c * PA, N1), :] = blk[:N1]
                    wnat[i, t, pl.ds((2 * c + 1) * PA, N1), :] = blk[N1:]

    dch = D // WCH
    for c in range(WCH):
        for i in range(3):
            copies[c * 3 + i].wait()

            def regroup(j, _, c=c, i=i):
                base = c * dch * NP + j
                a = wraw[i, pl.ds(base, dch // 2, stride=2 * NP), :]
                b = wraw[i, pl.ds(base + NP, dch // 2, stride=2 * NP), :]
                r = pl.ds(c * dch // 2, dch // 2)
                wqkv[j, r, pl.ds(i * 256, 128)] = (a & 0xFFFF) | (b << 16)
                wqkv[j, r, pl.ds(i * 256 + 128, 128)] = (a >> 16) | (b & np.uint32(0xFFFF0000))
            jax.lax.fori_loop(0, NP, regroup, None)
    for cp in loads[2 + 3 * WCH:]:
        cp.start()
    wo_cp.wait()
    x_cp.wait()

    ri = jax.lax.broadcasted_iota(jnp.int32, (2 * L, 2 * L), 0)
    ci = jax.lax.broadcasted_iota(jnp.int32, (2 * L, 2 * L), 1)
    same = (ri < L) == (ci < L)
    rl = jnp.where(ri < L, ri, ri - L)
    cl = jnp.where(ci < L, ci, ci - L)
    keep = same & ((rl < M) | (rl >= cl))
    fill = jnp.where(same, -1e9 * LOG2E, -jnp.inf).astype(F32)

    def layer(l, carry):
        def fetch(s):
            r = pl.ds(s * PX, SEG)
            x = jnp.where(l == 0, xin[jnp.minimum(s, NSEG - 1)].astype(F32), _ld(xs, r))
            _st(xs, r, x)
            hbuf[M:L, :] = _ln(x)

        def norm(s):
            r = pl.ds(s * PX, SEG)
            _st(hz, r, _ln(_ld(xs, r)))

        hbuf[0:M, :] = mem0_ref[...].astype(F32)
        fetch(0)

        def seg(s):
            r = pl.ds(s * PX, SEG)
            norm(jnp.maximum(s - 1, 0))
            st = {}

            def stack(a, o):
                return jnp.concatenate([a[:, o:o + 128], a[:, o + 128:o + 256]], axis=0)

            def proj_qk(j):
                a = _dot(hbuf[...], pltpu.bitcast(wqkv[j, :, 0:512], BF16))
                st["q", j], st["k", j] = stack(a, 0), stack(a, 256).astype(BF16)

            def proj_v(j):
                st["v", j] = stack(_dot(hbuf[...], pltpu.bitcast(wqkv[j, :, 512:768], BF16)), 0).astype(BF16)

            def scores(j):
                t = _dot_nt(st.pop(("q", j)), st.pop(("k", j))) * (DH ** -0.5 * LOG2E)
                t = jnp.where(keep, t, fill)
                e = jnp.exp2(t - jnp.max(t, axis=-1, keepdims=True))
                st["p", j] = e / jnp.sum(e, axis=-1, keepdims=True)

            def pv(j):
                o = _dot(st.pop(("p", j)), st.pop(("v", j)))
                obuf[:, j * 256:j * 256 + 128] = o[:L]
                obuf[:, j * 256 + 128:(j + 1) * 256] = o[L:]

            def proj_o(a, b):
                return _dot(obuf[:, a * 256:b * 256], pltpu.bitcast(wo32[a * 128:b * 128, :], BF16))

            y = None
            for op, *arg in _schedule():
                if op == "o":
                    y = proj_o(*arg) if y is None else y + proj_o(*arg)
                elif op == "gate":
                    z = (s // NSEG) * 8
                    for n, j in enumerate(arg):
                        gate[n, 0:2 * L, 0:2 * L] = st.pop(("p", j))
                    _st(gate.at[0:NT], pl.ds(2 * L, L), y)
                    for n, j in enumerate(arg):
                        st["p", j] = gate[n, pl.ds(z, 2 * L), 0:2 * L]
                elif op == "h":
                    fetch(s + 1)
                else:
                    {"qk": proj_qk, "v": proj_v, "s": scores, "pv": pv}[op](*arg)
            _st(xs, r, _rnd(_ld(xs, r) + y[M:]))
            hbuf[0:M, :] = y[:M]

        def segs(i, _):
            pl.when(l * NSEG + i == 1)(xt_cp.wait)
            for u in range(USEG):
                seg(i * USEG + u)
        jax.lax.fori_loop(0, NSEG // USEG, segs, None)
        norm(NSEG - 1)

        @pl.when(l == 0)
        def _():
            for cp in late_cp:
                cp.wait()
            filter_prep()

        def skew(n, first, second):
            prev = first(0)
            for u in range(n):
                nxt = first(u + 1) if u + 1 < n else None
                second(u, prev)
                prev = nxt

        tile = lambda a, t: a[:, t * 128:(t + 1) * 128]

        def fwd(i, _):
            def feat(u):
                r = pl.ds(i * UN + u, N1, stride=PX)
                z0, z1, z2, z3, z4 = (hz[t, r, :] for t in range(NT))
                s1, d1, s2, d2 = z1 + z4, z1 - z4, z2 + z3, z2 - z3
                u1 = jnp.concatenate([z0 + C1 * s1 + C2 * s2, -S1 * d1 - S2 * d2], axis=1)
                u2 = jnp.concatenate([z0 + C2 * s1 + C1 * s2, S1 * d2 - S2 * d1], axis=1)
                xf = [_dot(z0 + s1 + s2, g0_ref[...]), _dot(u1, g_ref[0]), _dot(u2, g_ref[1])]
                return jnp.concatenate(
                    [jnp.concatenate([tile(a, c) for a in xf], axis=1) for c in range(2)],
                    axis=0).astype(BF16)

            def seq(u, zf):
                n2 = i * UN + u
                a = _dot(m1_ref[n2], zf)
                _st(bufa, pl.ds(n2, N1, stride=PA), a[:N1])
                _st(bufa, pl.ds(n2 + N2, N1, stride=PA), a[N1:])
            skew(UN, feat, seq)
        jax.lax.fori_loop(0, N2 // UN, fwd, None)

        def mid(i, _):
            rows = lambda u, w: pl.ds((2 * (i * UN + u) + w) * PA, 2 * N2)

            def f2(u):
                a = jnp.concatenate([_ld(bufa, rows(u, 0)), _ld(bufa, rows(u, 1))], axis=0)
                xf = _dot(m2_ref[...], a.astype(BF16))
                ys = []
                for w in range(2):
                    kr = pl.ds(2 * (i * UN + u) + w, N2, stride=PA)
                    wr, wi = _ld(wnat.at[0], kr), _ld(wnat.at[1], kr)
                    xr, xi = xf[w * 64:w * 64 + 32], xf[w * 64 + 32:w * 64 + 64]
                    ys += [xr * wr - xi * wi, xr * wi + xi * wr]
                return jnp.concatenate(ys, axis=0).astype(BF16)

            def i2(u, y):
                b = _dot(m2t_ref[...], y)
                _st(bufb, rows(u, 0), b[:64])
                _st(bufb, rows(u, 1), b[64:])
            skew(UN, f2, i2)
        jax.lax.fori_loop(0, N1 // 2 // UN, mid, None)

        def inv(i, _):
            def seq(u):
                n2 = i * UN + u
                b = jnp.concatenate([_ld(bufb, pl.ds(n2, N1, stride=PA)),
                                     _ld(bufb, pl.ds(n2 + N2, N1, stride=PA))], axis=0)
                return _dot(m1t_ref[n2], b.astype(BF16)).astype(BF16)

            def feat(u, yf):
                ri_ = lambda t: jnp.concatenate([tile(yf[:N1], t), tile(yf[N1:], t)], axis=1)
                v0 = _dot(ri_(0), g0t_ref[...])
                v1, v2 = _dot(ri_(1), gt_ref[0]), _dot(ri_(2), gt_ref[1])
                a1, b1, a2, b2 = tile(v1, 0), tile(v1, 1), tile(v2, 0), tile(v2, 1)
                s1, s2 = v0 + C1 * a1 + C2 * a2, v0 + C2 * a1 + C1 * a2
                d1, d2 = -S1 * b1 - S2 * b2, S1 * b2 - S2 * b1
                y = jnp.concatenate([v0 + a1 + a2, s1 + d1, s2 + d2, s2 - d2, s1 - d1], axis=1)
                r = pl.ds(i * UN + u, N1, stride=PX)
                _st(xs, r, _rnd(_ld(xs, r) + y))
            skew(UN, seq, feat)

            for c, cp in enumerate(out_cp):
                @pl.when(l * len(out_cp) + i == len(out_cp) + c)
                def _():
                    for n1 in range(N1):
                        xout[c, n1] = _ld(xs, pl.ds(n1 * PX + c * UN, UN)).astype(BF16)
                    cp.start()
        jax.lax.fori_loop(0, N2 // UN, inv, None)
        return carry
    jax.lax.fori_loop(0, 2, layer, 0)

    for cp in out_cp:
        cp.wait()


@functools.partial(jax.jit, static_argnames=("A_seg_len",))
def pallas_interleave_layers__memory_aug_recurrent_mem_tr__spectral_gfnet__prompt_kernel(
    A_x, A_mem0, A_Wq, A_Wk, A_Wv, A_Wo, A_seg_len, B_x, B_w_r, B_w_i,
):
    del B_x
    assert A_seg_len == SEG and A_x.shape == (1, S, D) and A_Wq.shape == (D, H, DH)
    vmem = pl.BlockSpec(memory_space=pltpu.VMEM)
    hbm = pl.BlockSpec(memory_space=pl.ANY)
    late = (B_w_r.T, B_w_i.T, *_consts())
    assert len(late) == NLATE
    out = pl.pallas_call(
        _kernel,
        out_shape=jax.ShapeDtypeStruct((N1, N2 // UN, UN, D), BF16),
        in_specs=[vmem] + [hbm] * (5 + NLATE),
        out_specs=hbm,
        scratch_shapes=[pltpu.VMEM(a.shape, a.dtype) for a in late] + [
            pltpu.VMEM((NSEG, SEG, D), BF16),
            pltpu.VMEM((N2 // UN, N1, UN, D), BF16),
            pltpu.VMEM((3, D * NP + 64, DH), U32),
            pltpu.VMEM((NP, D // 2, 768), U32),
            pltpu.VMEM((H * DH // 2, D), U32),
            pltpu.VMEM((NT, (NSEG + 2) * PX, 128), F32),
            pltpu.VMEM((NT, (NSEG + 2) * PX, 128), F32),
            pltpu.VMEM((L, D), F32),
            pltpu.VMEM((NT, 3 * L, 128), F32),
            pltpu.VMEM((L, H * DH), F32),
            pltpu.VMEM((NF, (N1 + 2) * PA, 128), F32),
            pltpu.VMEM((NF, (N1 + 2) * PA, 128), F32),
            pltpu.VMEM((S // 128, DF + 7, 128), F32),
            pltpu.VMEM((2, NF, (N2 + 2) * PA, 128), F32),
            pltpu.SemaphoreType.DMA((3 * WCH + 3 + NLATE + N2 // UN,)),
        ],
        compiler_params=pltpu.CompilerParams(vmem_limit_bytes=110 * 1024 * 1024),
    )(A_mem0.reshape(M, D), A_x.reshape(NSEG, SEG, D),
      A_Wq.reshape(D * H, DH), A_Wk.reshape(D * H, DH), A_Wv.reshape(D * H, DH),
      A_Wo.reshape(H * DH, D), *late)
    return out.reshape(1, S, D)
```

```python
import functools

import numpy as np
import jax
import jax.numpy as jnp
import jax.experimental.pallas as pl
import jax.experimental.pallas.tpu as pltpu

F32 = jnp.float32
BF16 = jnp.bfloat16
U32 = jnp.uint32

S, D, H, DH, M, SEG = 2048, 640, 32, 128, 8, 32
L = M + SEG
NSEG = S // SEG
NT = D // 128
DF = D // 2 + 1
FP = 384
NF = FP // 128
N1, N2 = 64, 32
NP = H // 2
LAG_V, LAG_P, NG, G0, G1 = 2, 4, 2, 2, 6
USEG = 3
XHEAD = USEG + 2
UN = 8
NLATE = 11
LOG2E = 1.4426950408889634
PX = SEG + 4
PA = 2 * N2 + 4
C1, C2 = float(np.cos(0.4 * np.pi)), float(np.cos(0.8 * np.pi))
S1, S2 = float(np.sin(0.4 * np.pi)), float(np.sin(0.8 * np.pi))
WCH = 5


def _consts():
    a = np.arange(128)[:, None]
    m = np.arange(64)
    f0 = np.concatenate([5 * np.arange(65), np.full(63, -1)])
    fs = [f0, np.concatenate([1 + 5 * m, 4 + 5 * m]), np.concatenate([2 + 5 * m, 3 + 5 * m])]
    g = []
    for r, f in enumerate(fs):
        f = f[None, :]
        th = 2.0 * np.pi * ((a * f) % D) / D
        c, s = np.cos(th), np.sin(th)
        if r == 0:
            g.append(np.concatenate([c * (f >= 0), -s * ((f > 0) & (f < DF - 1))], axis=1))
        else:
            sg = np.where(f % 5 == r, 1.0, -1.0)
            g.append(np.block([[c, -s], [sg * s, sg * c]]))
    f = np.concatenate(fs)[None, :]

    k1 = np.arange(N1)[None, :, None]
    n1 = np.arange(N1)[None, None, :]
    n2 = np.arange(N2)[:, None, None]
    th = 2.0 * np.pi * (((N2 * n1 + n2) * k1) % S) / S
    c, s = np.cos(th), np.sin(th)
    m1 = np.concatenate([np.concatenate([c, s], 2), np.concatenate([-s, c], 2)], 1)

    k2 = np.arange(N2)[:, None]
    n2 = np.arange(N2)[None, :]
    th = 2.0 * np.pi * ((k2 * n2) % N2) / N2
    c, s = np.cos(th), np.sin(th)
    m2 = np.kron(np.eye(2), np.block([[c, s], [-s, c]]))

    cf = np.where((f == 0) | (f == DF - 1), 1.0, 2.0) * (f >= 0) / (S * D)
    as_bf = lambda a: np.ascontiguousarray(a).astype(np.float32).astype(BF16)
    return (as_bf(g[0]), as_bf(g[0].T), as_bf(np.stack(g[1:])),
            as_bf(np.stack([x.T for x in g[1:]])), as_bf(m1), as_bf(m1.transpose(0, 2, 1)),
            as_bf(m2), as_bf(m2.T), cf.astype(np.float32))


def _schedule():
    ops = [("qk", 0)]
    for j in range(NP + LAG_P):
        if j + 1 < NP:
            ops.append(("qk", j + 1))
        if j < NP:
            ops.append(("s", j))
        if 0 <= j - LAG_V < NP:
            ops.append(("v", j - LAG_V))
        if j - LAG_V == NP - 1:
            ops.append(("h",))
        if j - LAG_P == NP - NG:
            ops += [("o", 0, G0), ("gate", *range(NP - NG, NP)), ("o", G0, G1)]
        if j - LAG_P >= 0:
            ops.append(("pv", j - LAG_P))
    return ops + [("o", G1, NP)]


def _dot(a, b):
    return jax.lax.dot_general(a, b, (((1,), (0,)), ((), ())), preferred_element_type=F32)


def _dot_nt(a, b):
    return jax.lax.dot_general(a, b, (((1,), (1,)), ((), ())), preferred_element_type=F32)


def _ln(x):
    m = jnp.mean(x, axis=-1, keepdims=True)
    xc = x - m
    v = jnp.mean(xc * xc, axis=-1, keepdims=True)
    return xc * jax.lax.rsqrt(v + 1e-5)


def _rnd(x):
    return x.astype(BF16).astype(F32)


def _ld(ref, rows):
    return jnp.concatenate([ref[t, rows, :] for t in range(ref.shape[0])], axis=1)


def _st(ref, rows, val):
    for t in range(ref.shape[0]):
        ref[t, rows, :] = val[:, t * 128:(t + 1) * 128]


def _kernel(mem0_ref, x_hbm, wq_hbm, wk_hbm, wv_hbm, wo_hbm, *refs):
    late_hbm, out_hbm, late = refs[:NLATE], refs[NLATE], refs[NLATE + 1:2 * NLATE + 1]
    (xin, xout, wraw, wqkv, wo32, xs, hz, hbuf, gate, obuf, bufa, bufb, wpad, wnat,
     sems) = refs[2 * NLATE + 1:]
    wr_ref, wi_ref, g0_ref, g0t_ref, g_ref, gt_ref, m1_ref, m1t_ref, m2_ref, m2t_ref, cf_ref = late

    rows = D * NP // WCH
    pairs = [(x_hbm.at[pl.ds(0, XHEAD)], xin.at[pl.ds(0, XHEAD)])]
    pairs += [(w.bitcast(U32).at[pl.ds(c * rows, rows)], wraw.at[i, pl.ds(c * rows, rows)])
              for c in range(WCH) for i, w in enumerate((wq_hbm, wk_hbm, wv_hbm))]
    tail = pl.ds(XHEAD, NSEG - XHEAD)
    pairs += [(wo_hbm.bitcast(U32), wo32), (x_hbm.at[tail], xin.at[tail])] + list(zip(late_hbm, late))
    loads = [pltpu.make_async_copy(a, b, sems.at[n]) for n, (a, b) in enumerate(pairs)]
    x_cp, wo_cp, copies = loads[0], loads[1 + 3 * WCH], loads[1:1 + 3 * WCH]
    xt_cp, late_cp = loads[2 + 3 * WCH], loads[3 + 3 * WCH:]
    out_cp = [pltpu.make_async_copy(xout.at[i], out_hbm.at[:, i], sems.at[len(loads) + i])
              for i in range(N2 // UN)]
    for cp in loads[:2 + 3 * WCH]:
        cp.start()

    def filter_prep():
        for i, w in enumerate((wr_ref, wi_ref)):
            for c in range(S // 128):
                wpad[c, pl.ds(DF - 1, 8), :] = jnp.zeros((8, 128), F32)
                wpad[c, pl.ds(0, DF), :] = w[:, c * 128:(c + 1) * 128].astype(F32)
            for c in range(S // 128):
                res = lambda r: wpad[c, pl.ds(r, 64, stride=5), :]
                top = jnp.concatenate(
                    [wpad[c, pl.ds(DF - 1, 8), :], jnp.zeros((56, 128), F32)], axis=0)
                for t, (lo, hi) in enumerate(((res(0), top), (res(1), res(4)), (res(2), res(3)))):
                    blk = jnp.concatenate([lo, hi], axis=0).T * cf_ref[:, t * 128:(t + 1) * 128]
                    wnat[i, t, pl.ds(2 * c * PA, N1), :] = blk[:N1]
                    wnat[i, t, pl.ds((2 * c + 1) * PA, N1), :] = blk[N1:]

    dch = D // WCH
    for c in range(WCH):
        for i in range(3):
            copies[c * 3 + i].wait()

            def regroup(j, _, c=c, i=i):
                base = c * dch * NP + j
                a = wraw[i, pl.ds(base, dch // 2, stride=2 * NP), :]
                b = wraw[i, pl.ds(base + NP, dch // 2, stride=2 * NP), :]
                r = pl.ds(c * dch // 2, dch // 2)
                wqkv[j, r, pl.ds(i * 256, 128)] = (a & 0xFFFF) | (b << 16)
                wqkv[j, r, pl.ds(i * 256 + 128, 128)] = (a >> 16) | (b & np.uint32(0xFFFF0000))
            jax.lax.fori_loop(0, NP, regroup, None)
    x_cp.wait()

    ri = jax.lax.broadcasted_iota(jnp.int32, (2 * L, 2 * L), 0)
    ci = jax.lax.broadcasted_iota(jnp.int32, (2 * L, 2 * L), 1)
    same = (ri < L) == (ci < L)
    rl = jnp.where(ri < L, ri, ri - L)
    cl = jnp.where(ci < L, ci, ci - L)
    keep = same & ((rl < M) | (rl >= cl))
    fill = jnp.where(same, -1e9 * LOG2E, -jnp.inf).astype(F32)

    def layer(l, carry):
        def fetch(s):
            r = pl.ds(s * PX, SEG)
            x = jnp.where(l == 0, xin[jnp.minimum(s, NSEG - 1)].astype(F32), _ld(xs, r))
            _st(xs, r, x)
            hbuf[M:L, :] = _ln(x)

        def norm(s):
            r = pl.ds(s * PX, SEG)
            _st(hz, r, _ln(_ld(xs, r)))

        hbuf[0:M, :] = mem0_ref[...].astype(F32)
        fetch(0)

        def seg(s, first=False):
            r = pl.ds(s * PX, SEG)
            if not first:
                norm(s - 1)
            st = {}

            def stack(a, o):
                return jnp.concatenate([a[:, o:o + 128], a[:, o + 128:o + 256]], axis=0)

            def proj_qk(j):
                a = _dot(hbuf[...], pltpu.bitcast(wqkv[j, :, 0:512], BF16))
                st["q", j], st["k", j] = stack(a, 0), stack(a, 256).astype(BF16)

            def proj_v(j):
                st["v", j] = stack(_dot(hbuf[...], pltpu.bitcast(wqkv[j, :, 512:768], BF16)), 0).astype(BF16)

            def scores(j):
                t = _dot_nt(st.pop(("q", j)), st.pop(("k", j))) * (DH ** -0.5 * LOG2E)
                t = jnp.where(keep, t, fill)
                e = jnp.exp2(t - jnp.max(t, axis=-1, keepdims=True))
                st["p", j] = e / jnp.sum(e, axis=-1, keepdims=True)

            def pv(j):
                o = _dot(st.pop(("p", j)), st.pop(("v", j)))
                obuf[:, j * 256:j * 256 + 128] = o[:L]
                obuf[:, j * 256 + 128:(j + 1) * 256] = o[L:]

            def proj_o(a, b):
                return _dot(obuf[:, a * 256:b * 256], pltpu.bitcast(wo32[a * 128:b * 128, :], BF16))

            y = None
            for op, *arg in _schedule():
                if op == "o":
                    if first and y is None:
                        @pl.when(l == 0)
                        def _():
                            wo_cp.wait()
                            for cp in loads[2 + 3 * WCH:]:
                                cp.start()
                    y = proj_o(*arg) if y is None else y + proj_o(*arg)
                elif op == "gate":
                    if first:
                        continue
                    z = (s // NSEG) * 8
                    for n, j in enumerate(arg):
                        gate[n, 0:2 * L, 0:2 * L] = st.pop(("p", j))
                    _st(gate.at[0:NT], pl.ds(2 * L, L), y)
                    for n, j in enumerate(arg):
                        st["p", j] = gate[n, pl.ds(z, 2 * L), 0:2 * L]
                elif op == "h":
                    fetch(s + 1)
                else:
                    {"qk": proj_qk, "v": proj_v, "s": scores, "pv": pv}[op](*arg)
            _st(xs, r, _rnd(_ld(xs, r) + y[M:]))
            hbuf[0:M, :] = y[:M]

        def segs(i, _):
            pl.when(l * NSEG + i == 1)(xt_cp.wait)
            for u in range(USEG):
                seg(i * USEG + u + 1)
        seg(0, first=True)
        jax.lax.fori_loop(0, (NSEG - 1) // USEG, segs, None)
        norm(NSEG - 1)

        @pl.when(l == 0)
        def _():
            for cp in late_cp:
                cp.wait()
            filter_prep()

        def skew(n, first, second):
            prev = first(0)
            for u in range(n):
                nxt = first(u + 1) if u + 1 < n else None
                second(u, prev)
                prev = nxt

        tile = lambda a, t: a[:, t * 128:(t + 1) * 128]

        def fwd(i, _):
            def feat(u):
                r = pl.ds(i * UN + u, N1, stride=PX)
                z0, z1, z2, z3, z4 = (hz[t, r, :] for t in range(NT))
                s1, d1, s2, d2 = z1 + z4, z1 - z4, z2 + z3, z2 - z3
                u1 = jnp.concatenate([z0 + C1 * s1 + C2 * s2, -S1 * d1 - S2 * d2], axis=1)
                u2 = jnp.concatenate([z0 + C2 * s1 + C1 * s2, S1 * d2 - S2 * d1], axis=1)
                xf = [_dot(z0 + s1 + s2, g0_ref[...]), _dot(u1, g_ref[0]), _dot(u2, g_ref[1])]
                return jnp.concatenate(
                    [jnp.concatenate([tile(a, c) for a in xf], axis=1) for c in range(2)],
                    axis=0).astype(BF16)

            def seq(u, zf):
                n2 = i * UN + u
                a = _dot(m1_ref[n2], zf)
                _st(bufa, pl.ds(n2, N1, stride=PA), a[:N1])
                _st(bufa, pl.ds(n2 + N2, N1, stride=PA), a[N1:])
            skew(UN, feat, seq)
        jax.lax.fori_loop(0, N2 // UN, fwd, None)

        def mid(i, _):
            rows = lambda u, w: pl.ds((2 * (i * UN + u) + w) * PA, 2 * N2)

            def f2(u):
                a = jnp.concatenate([_ld(bufa, rows(u, 0)), _ld(bufa, rows(u, 1))], axis=0)
                xf = _dot(m2_ref[...], a.astype(BF16))
                ys = []
                for w in range(2):
                    kr = pl.ds(2 * (i * UN + u) + w, N2, stride=PA)
                    wr, wi = _ld(wnat.at[0], kr), _ld(wnat.at[1], kr)
                    xr, xi = xf[w * 64:w * 64 + 32], xf[w * 64 + 32:w * 64 + 64]
                    ys += [xr * wr - xi * wi, xr * wi + xi * wr]
                return jnp.concatenate(ys, axis=0).astype(BF16)

            def i2(u, y):
                b = _dot(m2t_ref[...], y)
                _st(bufb, rows(u, 0), b[:64])
                _st(bufb, rows(u, 1), b[64:])
            skew(UN, f2, i2)
        jax.lax.fori_loop(0, N1 // 2 // UN, mid, None)

        def inv(i, _):
            def seq(u):
                n2 = i * UN + u
                b = jnp.concatenate([_ld(bufb, pl.ds(n2, N1, stride=PA)),
                                     _ld(bufb, pl.ds(n2 + N2, N1, stride=PA))], axis=0)
                return _dot(m1t_ref[n2], b.astype(BF16)).astype(BF16)

            def feat(u, yf):
                ri_ = lambda t: jnp.concatenate([tile(yf[:N1], t), tile(yf[N1:], t)], axis=1)
                v0 = _dot(ri_(0), g0t_ref[...])
                v1, v2 = _dot(ri_(1), gt_ref[0]), _dot(ri_(2), gt_ref[1])
                a1, b1, a2, b2 = tile(v1, 0), tile(v1, 1), tile(v2, 0), tile(v2, 1)
                s1, s2 = v0 + C1 * a1 + C2 * a2, v0 + C2 * a1 + C1 * a2
                d1, d2 = -S1 * b1 - S2 * b2, S1 * b2 - S2 * b1
                y = jnp.concatenate([v0 + a1 + a2, s1 + d1, s2 + d2, s2 - d2, s1 - d1], axis=1)
                r = pl.ds(i * UN + u, N1, stride=PX)
                _st(xs, r, _rnd(_ld(xs, r) + y))
            skew(UN, seq, feat)

            for c, cp in enumerate(out_cp):
                @pl.when(l * len(out_cp) + i == len(out_cp) + c)
                def _():
                    for n1 in range(N1):
                        xout[c, n1] = _ld(xs, pl.ds(n1 * PX + c * UN, UN)).astype(BF16)
                    cp.start()
        jax.lax.fori_loop(0, N2 // UN, inv, None)
        return carry
    jax.lax.fori_loop(0, 2, layer, 0)

    for cp in out_cp:
        cp.wait()


@functools.partial(jax.jit, static_argnames=("A_seg_len",))
def pallas_interleave_layers__memory_aug_recurrent_mem_tr__spectral_gfnet__prompt_kernel(
    A_x, A_mem0, A_Wq, A_Wk, A_Wv, A_Wo, A_seg_len, B_x, B_w_r, B_w_i,
):
    del B_x
    assert A_seg_len == SEG and A_x.shape == (1, S, D) and A_Wq.shape == (D, H, DH)
    vmem = pl.BlockSpec(memory_space=pltpu.VMEM)
    hbm = pl.BlockSpec(memory_space=pl.ANY)
    late = (B_w_r.T, B_w_i.T, *_consts())
    assert len(late) == NLATE
    out = pl.pallas_call(
        _kernel,
        out_shape=jax.ShapeDtypeStruct((N1, N2 // UN, UN, D), BF16),
        in_specs=[vmem] + [hbm] * (5 + NLATE),
        out_specs=hbm,
        scratch_shapes=[pltpu.VMEM(a.shape, a.dtype) for a in late] + [
            pltpu.VMEM((NSEG, SEG, D), BF16),
            pltpu.VMEM((N2 // UN, N1, UN, D), BF16),
            pltpu.VMEM((3, D * NP + 64, DH), U32),
            pltpu.VMEM((NP, D // 2, 768), U32),
            pltpu.VMEM((H * DH // 2, D), U32),
            pltpu.VMEM((NT, (NSEG + 2) * PX, 128), F32),
            pltpu.VMEM((NT, (NSEG + 2) * PX, 128), F32),
            pltpu.VMEM((L, D), F32),
            pltpu.VMEM((NT, 3 * L, 128), F32),
            pltpu.VMEM((L, H * DH), F32),
            pltpu.VMEM((NF, (N1 + 2) * PA, 128), F32),
            pltpu.VMEM((NF, (N1 + 2) * PA, 128), F32),
            pltpu.VMEM((S // 128, DF + 7, 128), F32),
            pltpu.VMEM((2, NF, (N2 + 2) * PA, 128), F32),
            pltpu.SemaphoreType.DMA((3 * WCH + 3 + NLATE + N2 // UN,)),
        ],
        compiler_params=pltpu.CompilerParams(vmem_limit_bytes=110 * 1024 * 1024),
    )(A_mem0.reshape(M, D), A_x.reshape(NSEG, SEG, D),
      A_Wq.reshape(D * H, DH), A_Wk.reshape(D * H, DH), A_Wv.reshape(D * H, DH),
      A_Wo.reshape(H * DH, D), *late)
    return out.reshape(1, S, D)
```

```python
import functools

import numpy as np
import jax
import jax.numpy as jnp
import jax.experimental.pallas as pl
import jax.experimental.pallas.tpu as pltpu

F32 = jnp.float32
BF16 = jnp.bfloat16
U32 = jnp.uint32

S, D, H, DH, M, SEG = 2048, 640, 32, 128, 8, 32
L = M + SEG
NSEG = S // SEG
NT = D // 128
DF = D // 2 + 1
FP = 384
NF = FP // 128
N1, N2 = 64, 32
NP = H // 2
LAG_V, LAG_P, NG, G0, G1 = 2, 4, 2, 2, 6
USEG, UPRE = 2, 3
NPRE = 28
assert NPRE % USEG == 0 and (NPRE - 1) % UPRE == 0
XHEAD = UPRE + 2
UN = 8
NLATE = 11
LOG2E = 1.4426950408889634
PX = SEG + 4
PA = 2 * N2 + 4
C1, C2 = float(np.cos(0.4 * np.pi)), float(np.cos(0.8 * np.pi))
S1, S2 = float(np.sin(0.4 * np.pi)), float(np.sin(0.8 * np.pi))
WCH = 5


def _consts():
    a = np.arange(128)[:, None]
    m = np.arange(64)
    f0 = np.concatenate([5 * np.arange(65), np.full(63, -1)])
    fs = [f0, np.concatenate([1 + 5 * m, 4 + 5 * m]), np.concatenate([2 + 5 * m, 3 + 5 * m])]
    g = []
    for r, f in enumerate(fs):
        f = f[None, :]
        th = 2.0 * np.pi * ((a * f) % D) / D
        c, s = np.cos(th), np.sin(th)
        if r == 0:
            g.append(np.concatenate([c * (f >= 0), -s * ((f > 0) & (f < DF - 1))], axis=1))
        else:
            sg = np.where(f % 5 == r, 1.0, -1.0)
            g.append(np.block([[c, -s], [sg * s, sg * c]]))
    f = np.concatenate(fs)[None, :]

    k1 = np.arange(N1)[None, :, None]
    n1 = np.arange(N1)[None, None, :]
    n2 = np.arange(N2)[:, None, None]
    th = 2.0 * np.pi * (((N2 * n1 + n2) * k1) % S) / S
    c, s = np.cos(th), np.sin(th)
    m1 = np.concatenate([np.concatenate([c, s], 2), np.concatenate([-s, c], 2)], 1)

    k2 = np.arange(N2)[:, None]
    n2 = np.arange(N2)[None, :]
    th = 2.0 * np.pi * ((k2 * n2) % N2) / N2
    c, s = np.cos(th), np.sin(th)
    m2 = np.kron(np.eye(2), np.block([[c, s], [-s, c]]))

    cf = np.where((f == 0) | (f == DF - 1), 1.0, 2.0) * (f >= 0) / (S * D)
    as_bf = lambda a: np.ascontiguousarray(a).astype(np.float32).astype(BF16)
    return (as_bf(g[0]), as_bf(g[0].T), as_bf(np.stack(g[1:])),
            as_bf(np.stack([x.T for x in g[1:]])), as_bf(m1), as_bf(m1.transpose(0, 2, 1)),
            as_bf(m2), as_bf(m2.T), cf.astype(np.float32))


def _schedule():
    ops = [("qk", 0)]
    for j in range(NP + LAG_P):
        if j + 1 < NP:
            ops.append(("qk", j + 1))
        if j < NP:
            ops.append(("s", j))
        if 0 <= j - LAG_V < NP:
            ops.append(("v", j - LAG_V))
        if j - LAG_V == NP - 1:
            ops.append(("h",))
        if j - LAG_P == NP - NG:
            ops += [("o", 0, G0), ("gate", *range(NP - NG, NP)), ("o", G0, G1)]
        if j - LAG_P >= 0:
            ops.append(("pv", j - LAG_P))
    return ops + [("o", G1, NP)]


def _dot(a, b):
    return jax.lax.dot_general(a, b, (((1,), (0,)), ((), ())), preferred_element_type=F32)


def _dot_nt(a, b):
    return jax.lax.dot_general(a, b, (((1,), (1,)), ((), ())), preferred_element_type=F32)


def _ln(x):
    m = jnp.mean(x, axis=-1, keepdims=True)
    xc = x - m
    v = jnp.mean(xc * xc, axis=-1, keepdims=True)
    return xc * jax.lax.rsqrt(v + 1e-5)


def _rnd(x):
    return x.astype(BF16).astype(F32)


def _ld(ref, rows):
    return jnp.concatenate([ref[t, rows, :] for t in range(ref.shape[0])], axis=1)


def _st(ref, rows, val):
    for t in range(ref.shape[0]):
        ref[t, rows, :] = val[:, t * 128:(t + 1) * 128]


def _kernel(mem0_ref, x_hbm, wq_hbm, wk_hbm, wv_hbm, wo_hbm, *refs):
    late_hbm, out_hbm, late = refs[:NLATE], refs[NLATE], refs[NLATE + 1:2 * NLATE + 1]
    (xin, xout, xpre, hpre, pre, wraw, wqkv, wo32, xs, hz, hbuf, gate, obuf, bufa, bufb, wpad, wnat,
     sems) = refs[2 * NLATE + 1:]
    wr_ref, wi_ref, g0_ref, g0t_ref, g_ref, gt_ref, m1_ref, m1t_ref, m2_ref, m2t_ref, cf_ref = late

    rows = D * NP // WCH
    pairs = [(x_hbm.at[pl.ds(0, NPRE), pl.ds(SEG - 8, 8)], xpre),
             (x_hbm.at[pl.ds(0, XHEAD)], xin.at[pl.ds(0, XHEAD)])]
    pairs += [(w.bitcast(U32).at[pl.ds(c * rows, rows)], wraw.at[i, pl.ds(c * rows, rows)])
              for c in range(WCH) for i, w in enumerate((wq_hbm, wk_hbm, wv_hbm))]
    tail = pl.ds(XHEAD, NSEG - XHEAD)
    pairs += [(wo_hbm.bitcast(U32), wo32), (x_hbm.at[tail], xin.at[tail])] + list(zip(late_hbm, late))
    loads = [pltpu.make_async_copy(a, b, sems.at[n]) for n, (a, b) in enumerate(pairs)]
    xp_cp, x_cp, wo_cp = loads[0], loads[1], loads[2 + 3 * WCH]
    xt_cp, late_cp = loads[3 + 3 * WCH], loads[4 + 3 * WCH:]
    out_cp = [pltpu.make_async_copy(xout.at[i], out_hbm.at[:, i], sems.at[len(loads) + i])
              for i in range(N2 // UN)]
    for cp in loads[:3 + 3 * WCH]:
        cp.start()

    def filter_prep():
        for i, w in enumerate((wr_ref, wi_ref)):
            for c in range(S // 128):
                wpad[c, pl.ds(DF - 1, 8), :] = jnp.zeros((8, 128), F32)
                wpad[c, pl.ds(0, DF), :] = w[:, c * 128:(c + 1) * 128].astype(F32)
            for c in range(S // 128):
                res = lambda r: wpad[c, pl.ds(r, 64, stride=5), :]
                top = jnp.concatenate(
                    [wpad[c, pl.ds(DF - 1, 8), :], jnp.zeros((56, 128), F32)], axis=0)
                for t, (lo, hi) in enumerate(((res(0), top), (res(1), res(4)), (res(2), res(3)))):
                    blk = jnp.concatenate([lo, hi], axis=0).T * cf_ref[:, t * 128:(t + 1) * 128]
                    wnat[i, t, pl.ds(2 * c * PA, N1), :] = blk[:N1]
                    wnat[i, t, pl.ds((2 * c + 1) * PA, N1), :] = blk[N1:]

    xp_cp.wait()
    for n in range(NPRE):
        _st(hpre, pl.ds(n * 8, 8), _ln(xpre[n].astype(F32)))

    def regroup(n, _, init):
        c, i = n // 3, n % 3
        pltpu.make_async_copy(pairs[2][0], wraw.at[i, pl.ds(c * rows, rows)], sems.at[2 + n]).wait()
        for j in range(NP):
            a = wraw[i, pl.ds(c * rows + j, 64, stride=2 * NP), :]
            b = wraw[i, pl.ds(c * rows + j + NP, 64, stride=2 * NP), :]
            w = jnp.concatenate([(a & 0xFFFF) | (b << 16),
                                 (a >> 16) | (b & np.uint32(0xFFFF0000))], axis=1)
            wqkv[j, i, pl.ds(pl.multiple_of(c * 64, 64), 64), :] = w
            t = _dot(hpre[c], pltpu.bitcast(w, BF16))
            pre[j, i] = t if init else pre[j, i] + t
    jax.lax.fori_loop(0, 3, functools.partial(regroup, init=True), None)
    jax.lax.fori_loop(3, 3 * WCH, functools.partial(regroup, init=False), None)
    x_cp.wait()

    ri = jax.lax.broadcasted_iota(jnp.int32, (2 * L, 2 * L), 0)
    ci = jax.lax.broadcasted_iota(jnp.int32, (2 * L, 2 * L), 1)
    same = (ri < L) == (ci < L)
    rl = jnp.where(ri < L, ri, ri - L)
    cl = jnp.where(ci < L, ci, ci - L)
    keep = same & ((rl < M) | (rl >= cl))
    fill = jnp.where(same, -1e9 * LOG2E, -jnp.inf).astype(F32)

    def fetch(l, s):
        r = pl.ds(s * PX, SEG)
        x = xin[jnp.minimum(s, NSEG - 1)].astype(F32)
        if not isinstance(l, int):
            x = jnp.where(l == 0, x, _ld(xs, r))
        _st(xs, r, x)
        hbuf[M:L, :] = _ln(x)

    def norm(s):
        r = pl.ds(s * PX, SEG)
        _st(hz, r, _ln(_ld(xs, r)))

    def seg(l, s, early=False, first=False):
        r = pl.ds(s * PX, SEG)
        if not first:
            norm(jnp.maximum(s - 1, 0))
        st = {}

        def stack(a, o):
            return jnp.concatenate([a[:, o:o + 128], a[:, o + 128:o + 256]], axis=0)

        def proj(j, parts):
            w = pltpu.bitcast(jnp.concatenate([wqkv[j, i] for i in parts], axis=1), BF16)
            if not early:
                return _dot(hbuf[...], w)
            done = [pre[j, i, pl.ds(pl.multiple_of(s * 8, 8), 8), :] for i in parts]
            return jnp.concatenate([_dot(hbuf[0:L - 8, :], w), jnp.concatenate(done, axis=1)], axis=0)

        def proj_qk(j):
            a = proj(j, (0, 1))
            st["q", j], st["k", j] = stack(a, 0), stack(a, 256).astype(BF16)

        def proj_v(j):
            st["v", j] = stack(proj(j, (2,)), 0).astype(BF16)

        def scores(j):
            t = _dot_nt(st.pop(("q", j)), st.pop(("k", j))) * (DH ** -0.5 * LOG2E)
            t = jnp.where(keep, t, fill)
            e = jnp.exp2(t - jnp.max(t, axis=-1, keepdims=True))
            st["p", j] = e / jnp.sum(e, axis=-1, keepdims=True)

        def pv(j):
            o = _dot(st.pop(("p", j)), st.pop(("v", j)))
            obuf[:, j * 256:j * 256 + 128] = o[:L]
            obuf[:, j * 256 + 128:(j + 1) * 256] = o[L:]

        def proj_o(a, b):
            return _dot(obuf[:, a * 256:b * 256], pltpu.bitcast(wo32[a * 128:b * 128, :], BF16))

        y = None
        for op, *arg in _schedule():
            if op == "o":
                if first and y is None:
                    wo_cp.wait()
                    for cp in loads[3 + 3 * WCH:]:
                        cp.start()
                y = proj_o(*arg) if y is None else y + proj_o(*arg)
            elif op == "gate":
                if first:
                    continue
                z = (s // NSEG) * 8
                for n, j in enumerate(arg):
                    gate[n, 0:2 * L, 0:2 * L] = st.pop(("p", j))
                _st(gate.at[0:NT], pl.ds(2 * L, L), y)
                for n, j in enumerate(arg):
                    st["p", j] = gate[n, pl.ds(z, 2 * L), 0:2 * L]
            elif op == "h":
                fetch(l, s + 1)
            else:
                {"qk": proj_qk, "v": proj_v, "s": scores, "pv": pv}[op](*arg)
        _st(xs, r, _rnd(_ld(xs, r) + y[M:]))
        hbuf[0:M, :] = y[:M]

    def start(l):
        hbuf[0:M, :] = mem0_ref[...].astype(F32)
        fetch(l, 0)

    def early_segs(i, _):
        pl.when(i == 1)(xt_cp.wait)
        for u in range(UPRE):
            seg(0, i * UPRE + u + 1, early=True)
    start(0)
    seg(0, 0, early=True, first=True)
    jax.lax.fori_loop(0, (NPRE - 1) // UPRE, early_segs, None)

    def layer(l, carry):
        pl.when(l == 1)(lambda: start(l))

        def segs(i, _):
            for u in range(USEG):
                seg(l, i * USEG + u)
        jax.lax.fori_loop((1 - l) * (NPRE // USEG), NSEG // USEG, segs, None)
        norm(NSEG - 1)

        @pl.when(l == 0)
        def _():
            for cp in late_cp:
                cp.wait()
            filter_prep()

        def skew(n, first, second):
            prev = first(0)
            for u in range(n):
                nxt = first(u + 1) if u + 1 < n else None
                second(u, prev)
                prev = nxt

        tile = lambda a, t: a[:, t * 128:(t + 1) * 128]

        def fwd(i, _):
            def feat(u):
                r = pl.ds(i * UN + u, N1, stride=PX)
                z0, z1, z2, z3, z4 = (hz[t, r, :] for t in range(NT))
                s1, d1, s2, d2 = z1 + z4, z1 - z4, z2 + z3, z2 - z3
                u1 = jnp.concatenate([z0 + C1 * s1 + C2 * s2, -S1 * d1 - S2 * d2], axis=1)
                u2 = jnp.concatenate([z0 + C2 * s1 + C1 * s2, S1 * d2 - S2 * d1], axis=1)
                xf = [_dot(z0 + s1 + s2, g0_ref[...]), _dot(u1, g_ref[0]), _dot(u2, g_ref[1])]
                return jnp.concatenate(
                    [jnp.concatenate([tile(a, c) for a in xf], axis=1) for c in range(2)],
                    axis=0).astype(BF16)

            def seq(u, zf):
                n2 = i * UN + u
                a = _dot(m1_ref[n2], zf)
                _st(bufa, pl.ds(n2, N1, stride=PA), a[:N1])
                _st(bufa, pl.ds(n2 + N2, N1, stride=PA), a[N1:])
            skew(UN, feat, seq)
        jax.lax.fori_loop(0, N2 // UN, fwd, None)

        def mid(i, _):
            rows = lambda u, w: pl.ds((2 * (i * UN + u) + w) * PA, 2 * N2)

            def f2(u):
                a = jnp.concatenate([_ld(bufa, rows(u, 0)), _ld(bufa, rows(u, 1))], axis=0)
                xf = _dot(m2_ref[...], a.astype(BF16))
                ys = []
                for w in range(2):
                    kr = pl.ds(2 * (i * UN + u) + w, N2, stride=PA)
                    wr, wi = _ld(wnat.at[0], kr), _ld(wnat.at[1], kr)
                    xr, xi = xf[w * 64:w * 64 + 32], xf[w * 64 + 32:w * 64 + 64]
                    ys += [xr * wr - xi * wi, xr * wi + xi * wr]
                return jnp.concatenate(ys, axis=0).astype(BF16)

            def i2(u, y):
                b = _dot(m2t_ref[...], y)
                _st(bufb, rows(u, 0), b[:64])
                _st(bufb, rows(u, 1), b[64:])
            skew(UN, f2, i2)
        jax.lax.fori_loop(0, N1 // 2 // UN, mid, None)

        def inv(i, _):
            def seq(u):
                n2 = i * UN + u
                b = jnp.concatenate([_ld(bufb, pl.ds(n2, N1, stride=PA)),
                                     _ld(bufb, pl.ds(n2 + N2, N1, stride=PA))], axis=0)
                return _dot(m1t_ref[n2], b.astype(BF16)).astype(BF16)

            def feat(u, yf):
                ri_ = lambda t: jnp.concatenate([tile(yf[:N1], t), tile(yf[N1:], t)], axis=1)
                v0 = _dot(ri_(0), g0t_ref[...])
                v1, v2 = _dot(ri_(1), gt_ref[0]), _dot(ri_(2), gt_ref[1])
                a1, b1, a2, b2 = tile(v1, 0), tile(v1, 1), tile(v2, 0), tile(v2, 1)
                s1, s2 = v0 + C1 * a1 + C2 * a2, v0 + C2 * a1 + C1 * a2
                d1, d2 = -S1 * b1 - S2 * b2, S1 * b2 - S2 * b1
                y = jnp.concatenate([v0 + a1 + a2, s1 + d1, s2 + d2, s2 - d2, s1 - d1], axis=1)
                r = pl.ds(i * UN + u, N1, stride=PX)
                _st(xs, r, _rnd(_ld(xs, r) + y))
            skew(UN, seq, feat)

            for c, cp in enumerate(out_cp):
                @pl.when(l * len(out_cp) + i == len(out_cp) + c)
                def _():
                    for n1 in range(N1):
                        xout[c, n1] = _ld(xs, pl.ds(n1 * PX + c * UN, UN)).astype(BF16)
                    cp.start()
        jax.lax.fori_loop(0, N2 // UN, inv, None)
        return carry
    jax.lax.fori_loop(0, 2, layer, 0)

    for cp in out_cp:
        cp.wait()


@functools.partial(jax.jit, static_argnames=("A_seg_len",))
def pallas_interleave_layers__memory_aug_recurrent_mem_tr__spectral_gfnet__prompt_kernel(
    A_x, A_mem0, A_Wq, A_Wk, A_Wv, A_Wo, A_seg_len, B_x, B_w_r, B_w_i,
):
    del B_x
    assert A_seg_len == SEG and A_x.shape == (1, S, D) and A_Wq.shape == (D, H, DH)
    vmem = pl.BlockSpec(memory_space=pltpu.VMEM)
    hbm = pl.BlockSpec(memory_space=pl.ANY)
    late = (B_w_r.T, B_w_i.T, *_consts())
    assert len(late) == NLATE
    out = pl.pallas_call(
        _kernel,
        out_shape=jax.ShapeDtypeStruct((N1, N2 // UN, UN, D), BF16),
        in_specs=[vmem] + [hbm] * (5 + NLATE),
        out_specs=hbm,
        scratch_shapes=[pltpu.VMEM(a.shape, a.dtype) for a in late] + [
            pltpu.VMEM((NSEG, SEG, D), BF16),
            pltpu.VMEM((N2 // UN, N1, UN, D), BF16),
            pltpu.VMEM((NPRE, 8, D), BF16),
            pltpu.VMEM((NT, NPRE * 8, 128), F32),
            pltpu.VMEM((NP, 3, NPRE * 8, 256), F32),
            pltpu.VMEM((3, D * NP + 64, DH), U32),
            pltpu.VMEM((NP, 3, D // 2, 256), U32),
            pltpu.VMEM((H * DH // 2, D), U32),
            pltpu.VMEM((NT, (NSEG + 2) * PX, 128), F32),
            pltpu.VMEM((NT, (NSEG + 2) * PX, 128), F32),
            pltpu.VMEM((L, D), F32),
            pltpu.VMEM((NT, 3 * L, 128), F32),
            pltpu.VMEM((L, H * DH), F32),
            pltpu.VMEM((NF, (N1 + 2) * PA, 128), F32),
            pltpu.VMEM((NF, (N1 + 2) * PA, 128), F32),
            pltpu.VMEM((S // 128, DF + 7, 128), F32),
            pltpu.VMEM((2, NF, (N2 + 2) * PA, 128), F32),
            pltpu.SemaphoreType.DMA((3 * WCH + 4 + NLATE + N2 // UN,)),
        ],
        compiler_params=pltpu.CompilerParams(vmem_limit_bytes=120 * 1024 * 1024),
    )(A_mem0.reshape(M, D), A_x.reshape(NSEG, SEG, D),
      A_Wq.reshape(D * H, DH), A_Wk.reshape(D * H, DH), A_Wv.reshape(D * H, DH),
      A_Wo.reshape(H * DH, D), *late)
    return out.reshape(1, S, D)
```

```python
import functools

import numpy as np
import jax
import jax.numpy as jnp
import jax.experimental.pallas as pl
import jax.experimental.pallas.tpu as pltpu

F32 = jnp.float32
BF16 = jnp.bfloat16
U32 = jnp.uint32

S, D, H, DH, M, SEG = 2048, 640, 32, 128, 8, 32
L = M + SEG
NSEG = S // SEG
NT = D // 128
DF = D // 2 + 1
FP = 384
NF = FP // 128
N1, N2 = 64, 32
NP = H // 2
LAG_V, LAG_P, NG, G0, G1 = 3, 5, 2, 2, 6
USEG, UPRE = 2, 3
NPRE = 28
assert NPRE % USEG == 0 and (NPRE - 1) % UPRE == 0 and (NSEG - NPRE) // USEG >= S // 128
XHEAD = UPRE + 2
UN = 16
NLATE = 11
LOG2E = 1.4426950408889634
PX = SEG + 4
PA = 2 * N2 + 4
C1, C2 = float(np.cos(0.4 * np.pi)), float(np.cos(0.8 * np.pi))
S1, S2 = float(np.sin(0.4 * np.pi)), float(np.sin(0.8 * np.pi))
WCH = 5


def _consts():
    a = np.arange(128)[:, None]
    m = np.arange(64)
    f0 = np.concatenate([5 * np.arange(65), np.full(63, -1)])
    fs = [f0, np.concatenate([1 + 5 * m, 4 + 5 * m]), np.concatenate([2 + 5 * m, 3 + 5 * m])]
    g = []
    for r, f in enumerate(fs):
        f = f[None, :]
        th = 2.0 * np.pi * ((a * f) % D) / D
        c, s = np.cos(th), np.sin(th)
        if r == 0:
            g.append(np.concatenate([c * (f >= 0), -s * ((f > 0) & (f < DF - 1))], axis=1))
        else:
            sg = np.where(f % 5 == r, 1.0, -1.0)
            g.append(np.block([[c, -s], [sg * s, sg * c]]))
    f = np.concatenate(fs)[None, :]

    k1 = np.arange(N1)[None, :, None]
    n1 = np.arange(N1)[None, None, :]
    n2 = np.arange(N2)[:, None, None]
    th = 2.0 * np.pi * (((N2 * n1 + n2) * k1) % S) / S
    c, s = np.cos(th), np.sin(th)
    m1 = np.concatenate([np.concatenate([c, s], 2), np.concatenate([-s, c], 2)], 1)

    k2 = np.arange(N2)[:, None]
    n2 = np.arange(N2)[None, :]
    th = 2.0 * np.pi * ((k2 * n2) % N2) / N2
    c, s = np.cos(th), np.sin(th)
    m2 = np.kron(np.eye(2), np.block([[c, s], [-s, c]]))

    cf = np.where((f == 0) | (f == DF - 1), 1.0, 2.0) * (f >= 0) / (S * D)
    as_bf = lambda a: np.ascontiguousarray(a).astype(np.float32).astype(BF16)
    return (as_bf(g[0]), as_bf(g[0].T), as_bf(np.stack(g[1:])),
            as_bf(np.stack([x.T for x in g[1:]])), as_bf(m1), as_bf(m1.transpose(0, 2, 1)),
            as_bf(m2), as_bf(m2.T), cf.astype(np.float32))


def _schedule():
    ops = [("qk", 0)]
    for j in range(NP + LAG_P):
        if j + 1 < NP:
            ops.append(("qk", j + 1))
        if j < NP:
            ops.append(("s", j))
        if 0 <= j - LAG_V < NP:
            ops.append(("v", j - LAG_V))
        if j - LAG_V == NP - 1:
            ops.append(("h",))
        if j - LAG_P == NP - NG:
            ops += [("o", 0, G0), ("gate", *range(NP - NG, NP)), ("o", G0, G1)]
        if j - LAG_P >= 0:
            ops.append(("pv", j - LAG_P))
    return ops + [("o", G1, NP)]


def _dot(a, b):
    return jax.lax.dot_general(a, b, (((1,), (0,)), ((), ())), preferred_element_type=F32)


def _dot_nt(a, b):
    return jax.lax.dot_general(a, b, (((1,), (1,)), ((), ())), preferred_element_type=F32)


def _ln(x):
    m = jnp.mean(x, axis=-1, keepdims=True)
    xc = x - m
    v = jnp.mean(xc * xc, axis=-1, keepdims=True)
    return xc * jax.lax.rsqrt(v + 1e-5)


def _rnd(x):
    return x.astype(BF16).astype(F32)


def _ld(ref, rows):
    return jnp.concatenate([ref[t, rows, :] for t in range(ref.shape[0])], axis=1)


def _st(ref, rows, val):
    for t in range(ref.shape[0]):
        ref[t, rows, :] = val[:, t * 128:(t + 1) * 128]


def _kernel(mem0_ref, x_hbm, wq_hbm, wk_hbm, wv_hbm, wo_hbm, *refs):
    late_hbm, out_hbm, late = refs[:NLATE], refs[NLATE], refs[NLATE + 1:2 * NLATE + 1]
    (xin, xout, xpre, hpre, pre, wraw, wqkv, wo32, xs, hz, hbuf, hb16, gate, obuf, bufa, bufb, wpad, wnat,
     sems) = refs[2 * NLATE + 1:]
    wr_ref, wi_ref, g0_ref, g0t_ref, g_ref, gt_ref, m1_ref, m1t_ref, m2_ref, m2t_ref, cf_ref = late

    rows = D * NP // WCH
    pairs = [(x_hbm.at[pl.ds(0, NPRE), pl.ds(SEG - 8, 8)], xpre),
             (x_hbm.at[pl.ds(0, XHEAD)], xin.at[pl.ds(0, XHEAD)])]
    pairs += [(w.bitcast(U32).at[pl.ds(c * rows, rows)], wraw.at[i, pl.ds(c * rows, rows)])
              for c in range(WCH) for i, w in enumerate((wq_hbm, wk_hbm, wv_hbm))]
    tail = pl.ds(XHEAD, NSEG - XHEAD)
    pairs += [(wo_hbm.bitcast(U32), wo32), (x_hbm.at[tail], xin.at[tail])] + list(zip(late_hbm, late))
    loads = [pltpu.make_async_copy(a, b, sems.at[n]) for n, (a, b) in enumerate(pairs)]
    xp_cp, x_cp, wo_cp = loads[0], loads[1], loads[2 + 3 * WCH]
    xt_cp, late_cp = loads[3 + 3 * WCH], loads[4 + 3 * WCH:]
    out_cp = [pltpu.make_async_copy(xout.at[i], out_hbm.at[:, i], sems.at[len(loads) + i])
              for i in range(N2 // UN)]
    for cp in loads[:3 + 3 * WCH]:
        cp.start()

    def filter_prep(c, z):
        for i, w in enumerate((wr_ref, wi_ref)):
            wpad[i, pl.ds(DF - 1, 8), :] = jnp.zeros((8, 128), F32)
            wpad[i, pl.ds(0, DF), :] = w[:, pl.ds(pl.multiple_of(c * 128, 128), 128)].astype(F32)
            wpad[i, pl.ds(DF + 7, 8), :] = obuf[0:8, H * DH - 128:]
            res = lambda r: wpad[i, pl.ds(r + z, 64, stride=5), :]
            top = jnp.concatenate([wpad[i, pl.ds(DF - 1, 8), :], jnp.zeros((56, 128), F32)], axis=0)
            for t, (lo, hi) in enumerate(((res(0), top), (res(1), res(4)), (res(2), res(3)))):
                blk = jnp.concatenate([lo, hi], axis=0).T * cf_ref[:, t * 128:(t + 1) * 128]
                wnat[i, t, pl.ds(2 * c * PA, N1), :] = blk[:N1]
                wnat[i, t, pl.ds((2 * c + 1) * PA, N1), :] = blk[N1:]

    xp_cp.wait()
    for n in range(NPRE):
        _st(hpre, pl.ds(n * 8, 8), _ln(xpre[n].astype(F32)))

    def regroup(n, _, init):
        c, i = n // 3, n % 3
        pltpu.make_async_copy(pairs[2][0], wraw.at[i, pl.ds(c * rows, rows)], sems.at[2 + n]).wait()
        for j in range(NP):
            a = wraw[i, pl.ds(c * rows + j, 64, stride=2 * NP), :]
            b = wraw[i, pl.ds(c * rows + j + NP, 64, stride=2 * NP), :]
            w = jnp.concatenate([(a & 0xFFFF) | (b << 16),
                                 (a >> 16) | (b & np.uint32(0xFFFF0000))], axis=1)
            wqkv[j, i, pl.ds(pl.multiple_of(c * 64, 64), 64), :] = w
            t = _dot(hpre[c], pltpu.bitcast(w, BF16))
            pre[j, i] = t if init else pre[j, i] + t
    jax.lax.fori_loop(0, 3, functools.partial(regroup, init=True), None)
    jax.lax.fori_loop(3, 3 * WCH, functools.partial(regroup, init=False), None)
    x_cp.wait()

    ri = jax.lax.broadcasted_iota(jnp.int32, (2 * L, 2 * L), 0)
    ci = jax.lax.broadcasted_iota(jnp.int32, (2 * L, 2 * L), 1)
    same = (ri < L) == (ci < L)
    rl = jnp.where(ri < L, ri, ri - L)
    cl = jnp.where(ci < L, ci, ci - L)
    keep = same & ((rl < M) | (rl >= cl))
    fill = jnp.where(same, -1e9 * LOG2E, -jnp.inf).astype(F32)

    def fetch(l, s):
        r = pl.ds(s * PX, SEG)
        x = xin[jnp.minimum(s, NSEG - 1)].astype(F32)
        if not isinstance(l, int):
            x = jnp.where(l == 0, x, _ld(xs, r))
        _st(xs, r, x)
        h = _ln(x)
        hbuf[0:8, :] = h[SEG - 8:]
        hbuf[8:SEG, :] = h[:SEG - 8]

    def norm(s):
        r = pl.ds(s * PX, SEG)
        _st(hz, r, _ln(_ld(xs, r)))

    def seg(l, s, early=False, first=False):
        r = pl.ds(s * PX, SEG)
        if not first:
            norm(jnp.maximum(s - 1, 0))
        st = {}
        if early:
            hb16[...] = pltpu.bitcast(hbuf[8:L, :].astype(BF16), U32)

        def stack(a, o):
            return jnp.concatenate([a[:, o:o + 128], a[:, o + 128:o + 256]], axis=0)

        def proj(j, parts):
            w = pltpu.bitcast(jnp.concatenate([wqkv[j, i] for i in parts], axis=1), BF16)
            if early:
                a = _dot(pltpu.bitcast(hb16[...], BF16), w)
                last = jnp.concatenate(
                    [pre[j, i, pl.ds(pl.multiple_of(s * 8, 8), 8), :] for i in parts], axis=1)
            else:
                a = _dot(hbuf[...], w)
                last, a = a[:8], a[8:]
            return jnp.concatenate([a[SEG - 8:], a[:SEG - 8], last], axis=0)

        def proj_qk(j):
            a = proj(j, (0, 1))
            st["q", j], st["k", j] = stack(a, 0), stack(a, 256).astype(BF16)

        def proj_v(j):
            st["v", j] = stack(proj(j, (2,)), 0).astype(BF16)

        def scores(j):
            t = _dot_nt(st.pop(("q", j)), st.pop(("k", j))) * (DH ** -0.5 * LOG2E)
            t = jnp.where(keep, t, fill)
            e = jnp.exp2(t - jnp.max(t, axis=-1, keepdims=True))
            st["p", j] = e / jnp.sum(e, axis=-1, keepdims=True)

        def pv(j):
            o = _dot(st.pop(("p", j)), st.pop(("v", j)))
            obuf[:, j * 256:j * 256 + 128] = o[:L]
            obuf[:, j * 256 + 128:(j + 1) * 256] = o[L:]

        def proj_o(a, b):
            return _dot(obuf[:, a * 256:b * 256], pltpu.bitcast(wo32[a * 128:b * 128, :], BF16))

        y = None
        for op, *arg in _schedule():
            if op == "o":
                if first and y is None:
                    wo_cp.wait()
                    for cp in loads[3 + 3 * WCH:]:
                        cp.start()
                y = proj_o(*arg) if y is None else y + proj_o(*arg)
            elif op == "gate":
                if first:
                    continue
                z = (s // NSEG) * 8
                for n, j in enumerate(arg):
                    gate[n, 0:2 * L, 0:2 * L] = st.pop(("p", j))
                _st(gate, pl.ds(2 * L, 8), y[:8])
                for n, j in enumerate(arg):
                    st["p", j] = gate[n, pl.ds(z, 2 * L), 0:2 * L]
            elif op == "h":
                fetch(l, s + 1)
            else:
                {"qk": proj_qk, "v": proj_v, "s": scores, "pv": pv}[op](*arg)
        _st(xs, r, _rnd(_ld(xs, r) + y[M:]))
        hbuf[SEG:L, :] = y[:M]

    def start(l):
        hbuf[SEG:L, :] = mem0_ref[...].astype(F32)
        fetch(l, 0)

    def early_segs(i, _):
        pl.when(i == 1)(xt_cp.wait)
        for u in range(UPRE):
            seg(0, i * UPRE + u + 1, early=True)
    start(0)
    seg(0, 0, early=True, first=True)
    jax.lax.fori_loop(0, (NPRE - 1) // UPRE, early_segs, None)
    for cp in late_cp:
        cp.wait()

    def layer(l, carry):
        pl.when(l == 1)(lambda: start(l))

        def segs(i, _):
            for u in range(USEG):
                seg(l, i * USEG + u)
            filter_prep(i % (S // 128), i // NSEG)
        jax.lax.fori_loop((1 - l) * (NPRE // USEG), NSEG // USEG, segs, None)
        norm(NSEG - 1)

        def skew(n, first, second):
            prev = first(0)
            for u in range(n):
                nxt = first(u + 1) if u + 1 < n else None
                second(u, prev)
                prev = nxt

        tile = lambda a, t: a[:, t * 128:(t + 1) * 128]

        def fwd(i, _):
            def feat(u):
                r = pl.ds(i * UN + u, N1, stride=PX)
                z0, z1, z2, z3, z4 = (hz[t, r, :] for t in range(NT))
                s1, d1, s2, d2 = z1 + z4, z1 - z4, z2 + z3, z2 - z3
                u1 = jnp.concatenate([z0 + C1 * s1 + C2 * s2, -S1 * d1 - S2 * d2], axis=1)
                u2 = jnp.concatenate([z0 + C2 * s1 + C1 * s2, S1 * d2 - S2 * d1], axis=1)
                xf = [_dot(z0 + s1 + s2, g0_ref[...]), _dot(u1, g_ref[0]), _dot(u2, g_ref[1])]
                return jnp.concatenate(
                    [jnp.concatenate([tile(a, c) for a in xf], axis=1) for c in range(2)],
                    axis=0).astype(BF16)

            def seq(u, zf):
                n2 = i * UN + u
                a = _dot(m1_ref[n2], zf)
                _st(bufa, pl.ds(n2, N1, stride=PA), a[:N1])
                _st(bufa, pl.ds(n2 + N2, N1, stride=PA), a[N1:])
            skew(UN, feat, seq)
        jax.lax.fori_loop(0, N2 // UN, fwd, None)

        def mid(i, _):
            rows = lambda u, w: pl.ds((2 * (i * UN + u) + w) * PA, 2 * N2)

            def f2(u):
                a = jnp.concatenate([_ld(bufa, rows(u, 0)), _ld(bufa, rows(u, 1))], axis=0)
                xf = _dot(m2_ref[...], a.astype(BF16))
                ys = []
                for w in range(2):
                    kr = pl.ds(2 * (i * UN + u) + w, N2, stride=PA)
                    wr, wi = _ld(wnat.at[0], kr), _ld(wnat.at[1], kr)
                    xr, xi = xf[w * 64:w * 64 + 32], xf[w * 64 + 32:w * 64 + 64]
                    ys += [xr * wr - xi * wi, xr * wi + xi * wr]
                return jnp.concatenate(ys, axis=0).astype(BF16)

            def i2(u, y):
                b = _dot(m2t_ref[...], y)
                _st(bufb, rows(u, 0), b[:64])
                _st(bufb, rows(u, 1), b[64:])
            skew(UN, f2, i2)
        jax.lax.fori_loop(0, N1 // 2 // UN, mid, None)

        def inv(i, _):
            def seq(u):
                n2 = i * UN + u
                b = jnp.concatenate([_ld(bufb, pl.ds(n2, N1, stride=PA)),
                                     _ld(bufb, pl.ds(n2 + N2, N1, stride=PA))], axis=0)
                return _dot(m1t_ref[n2], b.astype(BF16)).astype(BF16)

            def feat(u, yf):
                ri_ = lambda t: jnp.concatenate([tile(yf[:N1], t), tile(yf[N1:], t)], axis=1)
                v0 = _dot(ri_(0), g0t_ref[...])
                v1, v2 = _dot(ri_(1), gt_ref[0]), _dot(ri_(2), gt_ref[1])
                a1, b1, a2, b2 = tile(v1, 0), tile(v1, 1), tile(v2, 0), tile(v2, 1)
                s1, s2 = v0 + C1 * a1 + C2 * a2, v0 + C2 * a1 + C1 * a2
                d1, d2 = -S1 * b1 - S2 * b2, S1 * b2 - S2 * b1
                y = jnp.concatenate([v0 + a1 + a2, s1 + d1, s2 + d2, s2 - d2, s1 - d1], axis=1)
                r = pl.ds(i * UN + u, N1, stride=PX)
                _st(xs, r, _rnd(_ld(xs, r) + y))
            skew(UN, seq, feat)

            for c, cp in enumerate(out_cp):
                @pl.when(l * len(out_cp) + i == len(out_cp) + c)
                def _():
                    for n1 in range(N1):
                        xout[c, n1] = _ld(xs, pl.ds(n1 * PX + c * UN, UN)).astype(BF16)
                    cp.start()
        jax.lax.fori_loop(0, N2 // UN, inv, None)
        return carry
    jax.lax.fori_loop(0, 2, layer, 0)

    for cp in out_cp:
        cp.wait()


@functools.partial(jax.jit, static_argnames=("A_seg_len",))
def pallas_interleave_layers__memory_aug_recurrent_mem_tr__spectral_gfnet__prompt_kernel(
    A_x, A_mem0, A_Wq, A_Wk, A_Wv, A_Wo, A_seg_len, B_x, B_w_r, B_w_i,
):
    del B_x
    assert A_seg_len == SEG and A_x.shape == (1, S, D) and A_Wq.shape == (D, H, DH)
    vmem = pl.BlockSpec(memory_space=pltpu.VMEM)
    hbm = pl.BlockSpec(memory_space=pl.ANY)
    late = (B_w_r.T, B_w_i.T, *_consts())
    assert len(late) == NLATE
    out = pl.pallas_call(
        _kernel,
        out_shape=jax.ShapeDtypeStruct((N1, N2 // UN, UN, D), BF16),
        in_specs=[vmem] + [hbm] * (5 + NLATE),
        out_specs=hbm,
        scratch_shapes=[pltpu.VMEM(a.shape, a.dtype) for a in late] + [
            pltpu.VMEM((NSEG, SEG, D), BF16),
            pltpu.VMEM((N2 // UN, N1, UN, D), BF16),
            pltpu.VMEM((NPRE, 8, D), BF16),
            pltpu.VMEM((NT, NPRE * 8, 128), F32),
            pltpu.VMEM((NP, 3, NPRE * 8, 256), F32),
            pltpu.VMEM((3, D * NP + 64, DH), U32),
            pltpu.VMEM((NP, 3, D // 2, 256), U32),
            pltpu.VMEM((H * DH // 2, D), U32),
            pltpu.VMEM((NT, (NSEG + 2) * PX, 128), F32),
            pltpu.VMEM((NT, (NSEG + 2) * PX, 128), F32),
            pltpu.VMEM((L, D), F32),
            pltpu.VMEM((SEG // 2, D), U32),
            pltpu.VMEM((NT, 2 * L + 16, 128), F32),
            pltpu.VMEM((L, H * DH), F32),
            pltpu.VMEM((NF, (N1 + 2) * PA, 128), F32),
            pltpu.VMEM((NF, (N1 + 2) * PA, 128), F32),
            pltpu.VMEM((2, DF + 15, 128), F32),
            pltpu.VMEM((2, NF, (N2 + 2) * PA, 128), F32),
            pltpu.SemaphoreType.DMA((3 * WCH + 4 + NLATE + N2 // UN,)),
        ],
        compiler_params=pltpu.CompilerParams(vmem_limit_bytes=120 * 1024 * 1024),
    )(A_mem0.reshape(M, D), A_x.reshape(NSEG, SEG, D),
      A_Wq.reshape(D * H, DH), A_Wk.reshape(D * H, DH), A_Wv.reshape(D * H, DH),
      A_Wo.reshape(H * DH, D), *late)
    return out.reshape(1, S, D)
```

```python
import functools

import numpy as np
import jax
import jax.numpy as jnp
import jax.experimental.pallas as pl
import jax.experimental.pallas.tpu as pltpu

F32 = jnp.float32
BF16 = jnp.bfloat16
U32 = jnp.uint32

S, D, H, DH, M, SEG = 2048, 640, 32, 128, 8, 32
L = M + SEG
NSEG = S // SEG
NT = D // 128
DF = D // 2 + 1
FP = 384
NF = FP // 128
N1, N2 = 64, 32
NP = H // 2
LAG_V, LAG_P, NG, G0, G1 = 3, 5, 2, 2, 6
USEG, UPRE = 2, 3
NPRE = 34
assert NPRE % USEG == 0 and (NPRE - 1) % UPRE == 0
XHEAD = UPRE + 2
UN = 16
NLATE = 11
LOG2E = 1.4426950408889634
PX = SEG + 4
PA = 2 * N2 + 4
PW = 2 * NP + 8
C1, C2 = float(np.cos(0.4 * np.pi)), float(np.cos(0.8 * np.pi))
S1, S2 = float(np.sin(0.4 * np.pi)), float(np.sin(0.8 * np.pi))
WCH = 5


def _consts():
    a = np.arange(128)[:, None]
    m = np.arange(64)
    f0 = np.concatenate([5 * np.arange(65), np.full(63, -1)])
    fs = [f0, np.concatenate([1 + 5 * m, 4 + 5 * m]), np.concatenate([2 + 5 * m, 3 + 5 * m])]
    g = []
    for r, f in enumerate(fs):
        f = f[None, :]
        th = 2.0 * np.pi * ((a * f) % D) / D
        c, s = np.cos(th), np.sin(th)
        if r == 0:
            g.append(np.concatenate([c * (f >= 0), -s * ((f > 0) & (f < DF - 1))], axis=1))
        else:
            sg = np.where(f % 5 == r, 1.0, -1.0)
            g.append(np.block([[c, -s], [sg * s, sg * c]]))
    f = np.concatenate(fs)[None, :]

    k1 = np.arange(N1)[None, :, None]
    n1 = np.arange(N1)[None, None, :]
    n2 = np.arange(N2)[:, None, None]
    th = 2.0 * np.pi * (((N2 * n1 + n2) * k1) % S) / S
    c, s = np.cos(th), np.sin(th)
    m1 = np.concatenate([np.concatenate([c, s], 2), np.concatenate([-s, c], 2)], 1)

    k2 = np.arange(N2)[:, None]
    n2 = np.arange(N2)[None, :]
    th = 2.0 * np.pi * ((k2 * n2) % N2) / N2
    c, s = np.cos(th), np.sin(th)
    m2 = np.kron(np.eye(2), np.block([[c, s], [-s, c]]))

    cf = np.where((f == 0) | (f == DF - 1), 1.0, 2.0) * (f >= 0) / (S * D)
    as_bf = lambda a: np.ascontiguousarray(a).astype(np.float32).astype(BF16)
    return (as_bf(g[0]), as_bf(g[0].T), as_bf(np.stack(g[1:])),
            as_bf(np.stack([x.T for x in g[1:]])), as_bf(m1), as_bf(m1.transpose(0, 2, 1)),
            as_bf(m2), as_bf(m2.T), cf.astype(np.float32))


def _schedule():
    ops = [("qk", 0)]
    for j in range(NP + LAG_P):
        if j + 1 < NP:
            ops.append(("qk", j + 1))
        if j < NP:
            ops.append(("s", j))
        if 0 <= j - LAG_V < NP:
            ops.append(("v", j - LAG_V))
        if j - LAG_V == NP - 1:
            ops.append(("h",))
        if j - LAG_P == NP - NG:
            ops += [("o", 0, G0), ("gate", *range(NP - NG, NP)), ("o", G0, G1)]
        if j - LAG_P >= 0:
            ops.append(("pv", j - LAG_P))
    return ops + [("o", G1, NP)]


def _dot(a, b):
    return jax.lax.dot_general(a, b, (((1,), (0,)), ((), ())), preferred_element_type=F32)


def _dot_nt(a, b):
    return jax.lax.dot_general(a, b, (((1,), (1,)), ((), ())), preferred_element_type=F32)


def _ln(x):
    m = jnp.mean(x, axis=-1, keepdims=True)
    xc = x - m
    v = jnp.mean(xc * xc, axis=-1, keepdims=True)
    return xc * jax.lax.rsqrt(v + 1e-5)


def _rnd(x):
    return x.astype(BF16).astype(F32)


def _ld(ref, rows):
    return jnp.concatenate([ref[t, rows, :] for t in range(ref.shape[0])], axis=1)


def _st(ref, rows, val):
    for t in range(ref.shape[0]):
        ref[t, rows, :] = val[:, t * 128:(t + 1) * 128]


def _kernel(mem0_ref, x_hbm, wq_hbm, wk_hbm, wv_hbm, wo_hbm, *refs):
    late_hbm, out_hbm, late = refs[:NLATE], refs[NLATE], refs[NLATE + 1:2 * NLATE + 1]
    (xin, xout, xpre, hpre, pre, wraw, wqkv, wo32, xs, hz, hbuf, hb16, gate, obuf, bufa, bufb, wpad, wnat,
     sems) = refs[2 * NLATE + 1:]
    wr_ref, wi_ref, g0_ref, g0t_ref, g_ref, gt_ref, m1_ref, m1t_ref, m2_ref, m2t_ref, cf_ref = late

    chunk = lambda n: wraw.at[pl.ds(n * 64, 64), pl.ds(0, 2 * NP)]
    pairs = [(x_hbm.at[pl.ds(0, NPRE), pl.ds(SEG - 8, 8)], xpre),
             (x_hbm.at[pl.ds(0, XHEAD)], xin.at[pl.ds(0, XHEAD)])]
    pairs += [(w.bitcast(U32).at[pl.ds(c * 64, 64)], chunk(3 * c + i))
              for c in range(WCH) for i, w in enumerate((wq_hbm, wk_hbm, wv_hbm))]
    tail = pl.ds(XHEAD, NSEG - XHEAD)
    pairs += [(wo_hbm.bitcast(U32), wo32), (x_hbm.at[tail], xin.at[tail])] + list(zip(late_hbm, late))
    loads = [pltpu.make_async_copy(a, b, sems.at[n]) for n, (a, b) in enumerate(pairs)]
    xp_cp, x_cp, wo_cp = loads[0], loads[1], loads[2 + 3 * WCH]
    xt_cp, late_cp = loads[3 + 3 * WCH], loads[4 + 3 * WCH:]
    out_cp = [pltpu.make_async_copy(xout.at[i], out_hbm.at[:, i], sems.at[len(loads) + i])
              for i in range(N2 // UN)]
    for cp in loads[:3 + 3 * WCH]:
        cp.start()

    def filter_prep(c, z):
        for i, w in enumerate((wr_ref, wi_ref)):
            wpad[i, pl.ds(DF - 1, 8), :] = jnp.zeros((8, 128), F32)
            wpad[i, pl.ds(0, DF), :] = w[:, pl.ds(pl.multiple_of(c * 128, 128), 128)].astype(F32)
            wpad[i, pl.ds(DF + 7, 8), :] = obuf[0:8, H * DH - 128:]
            res = lambda r: wpad[i, pl.ds(r + z, 64, stride=5), :]
            top = jnp.concatenate([wpad[i, pl.ds(DF - 1, 8), :], jnp.zeros((56, 128), F32)], axis=0)
            for t, (lo, hi) in enumerate(((res(0), top), (res(1), res(4)), (res(2), res(3)))):
                blk = jnp.concatenate([lo, hi], axis=0).T * cf_ref[:, t * 128:(t + 1) * 128]
                wnat[i, t, pl.ds(2 * c * PA, N1), :] = blk[:N1]
                wnat[i, t, pl.ds((2 * c + 1) * PA, N1), :] = blk[N1:]

    xp_cp.wait()
    for n in range(NPRE):
        _st(hpre, pl.ds(n * 8, 8), _ln(xpre[n].astype(F32)))

    wflat = wraw.reshape(wraw.shape[0] * PW, DH)

    def regroup(n, _, init):
        c, i = n // 3, n % 3
        pltpu.make_async_copy(pairs[2][0], chunk(n), sems.at[2 + n]).wait()
        for j in range(NP):
            a = wflat[pl.ds(n * 64 * PW + j, 64, stride=PW), :]
            b = wflat[pl.ds(n * 64 * PW + j + NP, 64, stride=PW), :]
            w = jnp.concatenate([(a & 0xFFFF) | (b << 16),
                                 (a >> 16) | (b & np.uint32(0xFFFF0000))], axis=1)
            wqkv[j, i, pl.ds(pl.multiple_of(c * 64, 64), 64), :] = w
            t = _dot(hpre[c], pltpu.bitcast(w, BF16))
            pre[j, i] = t if init else pre[j, i] + t
    jax.lax.fori_loop(0, 3, functools.partial(regroup, init=True), None)
    jax.lax.fori_loop(3, 3 * WCH, functools.partial(regroup, init=False), None)
    x_cp.wait()

    ri = jax.lax.broadcasted_iota(jnp.int32, (2 * L, 2 * L), 0)
    ci = jax.lax.broadcasted_iota(jnp.int32, (2 * L, 2 * L), 1)
    same = (ri < L) == (ci < L)
    rl = jnp.where(ri < L, ri, ri - L)
    cl = jnp.where(ci < L, ci, ci - L)
    keep = same & ((rl < M) | (rl >= cl))
    fill = jnp.where(same, -1e9 * LOG2E, -jnp.inf).astype(F32)

    def fetch(l, s):
        r = pl.ds(s * PX, SEG)
        x = xin[jnp.minimum(s, NSEG - 1)].astype(F32)
        if not isinstance(l, int):
            x = jnp.where(l == 0, x, _ld(xs, r))
        _st(xs, r, x)
        h = _ln(x)
        hbuf[0:8, :] = h[SEG - 8:]
        hbuf[8:SEG, :] = h[:SEG - 8]

    def norm(s):
        r = pl.ds(s * PX, SEG)
        _st(hz, r, _ln(_ld(xs, r)))

    def seg(l, s, early=False, first=False):
        r = pl.ds(s * PX, SEG)
        if not first:
            norm(jnp.maximum(s - 1, 0))
        st = {}
        if early:
            hb16[...] = pltpu.bitcast(hbuf[8:L, :].astype(BF16), U32)

        def stack(a, o):
            return jnp.concatenate([a[:, o:o + 128], a[:, o + 128:o + 256]], axis=0)

        def proj(j, parts):
            w = pltpu.bitcast(jnp.concatenate([wqkv[j, i] for i in parts], axis=1), BF16)
            if early:
                a = _dot(pltpu.bitcast(hb16[...], BF16), w)
                last = jnp.concatenate(
                    [pre[j, i, pl.ds(pl.multiple_of(s * 8, 8), 8), :] for i in parts], axis=1)
            else:
                a = _dot(hbuf[...], w)
                last, a = a[:8], a[8:]
            return jnp.concatenate([a[SEG - 8:], a[:SEG - 8], last], axis=0)

        def proj_qk(j):
            a = proj(j, (0, 1))
            st["q", j], st["k", j] = stack(a, 0), stack(a, 256).astype(BF16)

        def proj_v(j):
            st["v", j] = stack(proj(j, (2,)), 0).astype(BF16)

        def scores(j):
            t = _dot_nt(st.pop(("q", j)), st.pop(("k", j))) * (DH ** -0.5 * LOG2E)
            t = jnp.where(keep, t, fill)
            e = jnp.exp2(t - jnp.max(t, axis=-1, keepdims=True))
            st["p", j] = e / jnp.sum(e, axis=-1, keepdims=True)

        def pv(j):
            o = _dot(st.pop(("p", j)), st.pop(("v", j)))
            obuf[:, j * 256:j * 256 + 128] = o[:L]
            obuf[:, j * 256 + 128:(j + 1) * 256] = o[L:]

        def proj_o(a, b):
            return _dot(obuf[:, a * 256:b * 256], pltpu.bitcast(wo32[a * 128:b * 128, :], BF16))

        y = None
        for op, *arg in _schedule():
            if op == "o":
                if first and y is None:
                    wo_cp.wait()
                    for cp in loads[3 + 3 * WCH:]:
                        cp.start()
                y = proj_o(*arg) if y is None else y + proj_o(*arg)
            elif op == "gate":
                if first:
                    continue
                z = (s // NSEG) * 8
                for n, j in enumerate(arg):
                    gate[n, 0:2 * L, 0:2 * L] = st.pop(("p", j))
                _st(gate, pl.ds(2 * L, 8), y[:8])
                for n, j in enumerate(arg):
                    st["p", j] = gate[n, pl.ds(z, 2 * L), 0:2 * L]
            elif op == "h":
                fetch(l, s + 1)
            else:
                {"qk": proj_qk, "v": proj_v, "s": scores, "pv": pv}[op](*arg)
        _st(xs, r, _rnd(_ld(xs, r) + y[M:]))
        hbuf[SEG:L, :] = y[:M]

    def start(l):
        hbuf[SEG:L, :] = mem0_ref[...].astype(F32)
        fetch(l, 0)

    def early_segs(i, _):
        pl.when(i == 1)(xt_cp.wait)
        for u in range(UPRE):
            seg(0, i * UPRE + u + 1, early=True)
    start(0)
    seg(0, 0, early=True, first=True)
    jax.lax.fori_loop(0, (NPRE - 1) // UPRE, early_segs, None)
    for cp in late_cp:
        cp.wait()
    for i in range(NSEG // USEG - S // 128, NPRE // USEG):
        filter_prep(i % (S // 128), 0)

    def layer(l, carry):
        pl.when(l == 1)(lambda: start(l))

        def segs(i, _):
            for u in range(USEG):
                seg(l, i * USEG + u)
            filter_prep(i % (S // 128), i // NSEG)
        jax.lax.fori_loop((1 - l) * (NPRE // USEG), NSEG // USEG, segs, None)
        norm(NSEG - 1)

        def skew(n, first, second):
            prev = first(0)
            for u in range(n):
                nxt = first(u + 1) if u + 1 < n else None
                second(u, prev)
                prev = nxt

        tile = lambda a, t: a[:, t * 128:(t + 1) * 128]

        def fwd(i, _):
            def feat(u):
                r = pl.ds(i * UN + u, N1, stride=PX)
                z0, z1, z2, z3, z4 = (hz[t, r, :] for t in range(NT))
                s1, d1, s2, d2 = z1 + z4, z1 - z4, z2 + z3, z2 - z3
                u1 = jnp.concatenate([z0 + C1 * s1 + C2 * s2, -S1 * d1 - S2 * d2], axis=1)
                u2 = jnp.concatenate([z0 + C2 * s1 + C1 * s2, S1 * d2 - S2 * d1], axis=1)
                xf = [_dot(z0 + s1 + s2, g0_ref[...]), _dot(u1, g_ref[0]), _dot(u2, g_ref[1])]
                return jnp.concatenate(
                    [jnp.concatenate([tile(a, c) for a in xf], axis=1) for c in range(2)],
                    axis=0).astype(BF16)

            def seq(u, zf):
                n2 = i * UN + u
                a = _dot(m1_ref[n2], zf)
                _st(bufa, pl.ds(n2, N1, stride=PA), a[:N1])
                _st(bufa, pl.ds(n2 + N2, N1, stride=PA), a[N1:])
            skew(UN, feat, seq)
        jax.lax.fori_loop(0, N2 // UN, fwd, None)

        def mid(i, _):
            rows = lambda u, w: pl.ds((2 * (i * UN + u) + w) * PA, 2 * N2)

            def f2(u):
                a = jnp.concatenate([_ld(bufa, rows(u, 0)), _ld(bufa, rows(u, 1))], axis=0)
                xf = _dot(m2_ref[...], a.astype(BF16))
                ys = []
                for w in range(2):
                    kr = pl.ds(2 * (i * UN + u) + w, N2, stride=PA)
                    wr, wi = _ld(wnat.at[0], kr), _ld(wnat.at[1], kr)
                    xr, xi = xf[w * 64:w * 64 + 32], xf[w * 64 + 32:w * 64 + 64]
                    ys += [xr * wr - xi * wi, xr * wi + xi * wr]
                return jnp.concatenate(ys, axis=0).astype(BF16)

            def i2(u, y):
                b = _dot(m2t_ref[...], y)
                _st(bufb, rows(u, 0), b[:64])
                _st(bufb, rows(u, 1), b[64:])
            skew(UN, f2, i2)
        jax.lax.fori_loop(0, N1 // 2 // UN, mid, None)

        def inv(i, _):
            def seq(u):
                n2 = i * UN + u
                b = jnp.concatenate([_ld(bufb, pl.ds(n2, N1, stride=PA)),
                                     _ld(bufb, pl.ds(n2 + N2, N1, stride=PA))], axis=0)
                return _dot(m1t_ref[n2], b.astype(BF16)).astype(BF16)

            def feat(u, yf):
                ri_ = lambda t: jnp.concatenate([tile(yf[:N1], t), tile(yf[N1:], t)], axis=1)
                v0 = _dot(ri_(0), g0t_ref[...])
                v1, v2 = _dot(ri_(1), gt_ref[0]), _dot(ri_(2), gt_ref[1])
                a1, b1, a2, b2 = tile(v1, 0), tile(v1, 1), tile(v2, 0), tile(v2, 1)
                s1, s2 = v0 + C1 * a1 + C2 * a2, v0 + C2 * a1 + C1 * a2
                d1, d2 = -S1 * b1 - S2 * b2, S1 * b2 - S2 * b1
                y = jnp.concatenate([v0 + a1 + a2, s1 + d1, s2 + d2, s2 - d2, s1 - d1], axis=1)
                r = pl.ds(i * UN + u, N1, stride=PX)
                _st(xs, r, _rnd(_ld(xs, r) + y))
            skew(UN, seq, feat)

            for c, cp in enumerate(out_cp):
                @pl.when(l * len(out_cp) + i == len(out_cp) + c)
                def _():
                    for n1 in range(N1):
                        xout[c, n1] = _ld(xs, pl.ds(n1 * PX + c * UN, UN)).astype(BF16)
                    cp.start()
        jax.lax.fori_loop(0, N2 // UN, inv, None)
        return carry
    jax.lax.fori_loop(0, 2, layer, 0)

    for cp in out_cp:
        cp.wait()


@functools.partial(jax.jit, static_argnames=("A_seg_len",))
def pallas_interleave_layers__memory_aug_recurrent_mem_tr__spectral_gfnet__prompt_kernel(
    A_x, A_mem0, A_Wq, A_Wk, A_Wv, A_Wo, A_seg_len, B_x, B_w_r, B_w_i,
):
    del B_x
    assert A_seg_len == SEG and A_x.shape == (1, S, D) and A_Wq.shape == (D, H, DH)
    vmem = pl.BlockSpec(memory_space=pltpu.VMEM)
    hbm = pl.BlockSpec(memory_space=pl.ANY)
    late = (B_w_r.T, B_w_i.T, *_consts())
    assert len(late) == NLATE
    out = pl.pallas_call(
        _kernel,
        out_shape=jax.ShapeDtypeStruct((N1, N2 // UN, UN, D), BF16),
        in_specs=[vmem] + [hbm] * (5 + NLATE),
        out_specs=hbm,
        scratch_shapes=[pltpu.VMEM(a.shape, a.dtype) for a in late] + [
            pltpu.VMEM((NSEG, SEG, D), BF16),
            pltpu.VMEM((N2 // UN, N1, UN, D), BF16),
            pltpu.VMEM((NPRE, 8, D), BF16),
            pltpu.VMEM((NT, NPRE * 8, 128), F32),
            pltpu.VMEM((NP, 3, NPRE * 8, 256), F32),
            pltpu.VMEM((3 * D // 2 + 1, PW, DH), U32),
            pltpu.VMEM((NP, 3, D // 2, 256), U32),
            pltpu.VMEM((H * DH // 2, D), U32),
            pltpu.VMEM((NT, (NSEG + 2) * PX, 128), F32),
            pltpu.VMEM((NT, (NSEG + 2) * PX, 128), F32),
            pltpu.VMEM((L, D), F32),
            pltpu.VMEM((SEG // 2, D), U32),
            pltpu.VMEM((NT, 2 * L + 16, 128), F32),
            pltpu.VMEM((L, H * DH), F32),
            pltpu.VMEM((NF, (N1 + 2) * PA, 128), F32),
            pltpu.VMEM((NF, (N1 + 2) * PA, 128), F32),
            pltpu.VMEM((2, DF + 15, 128), F32),
            pltpu.VMEM((2, NF, (N2 + 2) * PA, 128), F32),
            pltpu.SemaphoreType.DMA((3 * WCH + 4 + NLATE + N2 // UN,)),
        ],
        compiler_params=pltpu.CompilerParams(vmem_limit_bytes=120 * 1024 * 1024),
    )(A_mem0.reshape(M, D), A_x.reshape(NSEG, SEG, D),
      A_Wq.reshape(D // 2, 2 * H, DH), A_Wk.reshape(D // 2, 2 * H, DH), A_Wv.reshape(D // 2, 2 * H, DH),
      A_Wo.reshape(H * DH, D), *late)
    return out.reshape(1, S, D)
```

```python
import functools

import numpy as np
import jax
import jax.numpy as jnp
import jax.experimental.pallas as pl
import jax.experimental.pallas.tpu as pltpu

F32 = jnp.float32
BF16 = jnp.bfloat16
U32 = jnp.uint32

S, D, H, DH, M, SEG = 2048, 640, 32, 128, 8, 32
L = M + SEG
NSEG = S // SEG
NT = D // 128
DF = D // 2 + 1
FP = 384
NF = FP // 128
N1, N2 = 64, 32
NP = H // 2
LAG_V, LAG_P, NG, G0, G1 = 3, 5, 2, 2, 6
USEG, UPRE = 2, 3
NPRE = 34
assert NPRE % USEG == 0 and (NPRE - 1) % UPRE == 0
XHEAD = UPRE + 2
UN = 16
NLATE = 11
LOG2E = 1.4426950408889634
PX = SEG + 4
PA = 2 * N2 + 4
PW = 2 * NP + 8
C1, C2 = float(np.cos(0.4 * np.pi)), float(np.cos(0.8 * np.pi))
S1, S2 = float(np.sin(0.4 * np.pi)), float(np.sin(0.8 * np.pi))
WCH = 5


def _consts():
    a = np.arange(128)[:, None]
    m = np.arange(64)
    f0 = np.concatenate([5 * np.arange(65), np.full(63, -1)])
    fs = [f0, np.concatenate([1 + 5 * m, 4 + 5 * m]), np.concatenate([2 + 5 * m, 3 + 5 * m])]
    g = []
    for r, f in enumerate(fs):
        f = f[None, :]
        th = 2.0 * np.pi * ((a * f) % D) / D
        c, s = np.cos(th), np.sin(th)
        if r == 0:
            g.append(np.concatenate([c * (f >= 0), -s * ((f > 0) & (f < DF - 1))], axis=1))
        else:
            sg = np.where(f % 5 == r, 1.0, -1.0)
            g.append(np.block([[c, -s], [sg * s, sg * c]]))
    f = np.concatenate(fs)[None, :]

    k1 = np.arange(N1)[None, :, None]
    n1 = np.arange(N1)[None, None, :]
    n2 = np.arange(N2)[:, None, None]
    th = 2.0 * np.pi * (((N2 * n1 + n2) * k1) % S) / S
    c, s = np.cos(th), np.sin(th)
    m1 = np.concatenate([np.concatenate([c, s], 2), np.concatenate([-s, c], 2)], 1)

    k2 = np.arange(N2)[:, None]
    n2 = np.arange(N2)[None, :]
    th = 2.0 * np.pi * ((k2 * n2) % N2) / N2
    c, s = np.cos(th), np.sin(th)
    m2 = np.kron(np.eye(2), np.block([[c, s], [-s, c]]))

    cf = np.where((f == 0) | (f == DF - 1), 1.0, 2.0) * (f >= 0) / (S * D)
    as_bf = lambda a: np.ascontiguousarray(a).astype(np.float32).astype(BF16)
    return (as_bf(g[0]), as_bf(g[0].T), as_bf(np.stack(g[1:])),
            as_bf(np.stack([x.T for x in g[1:]])), as_bf(m1), as_bf(m1.transpose(0, 2, 1)),
            as_bf(m2), as_bf(m2.T), cf.astype(np.float32))


def _schedule():
    ops = [("qk", 0)]
    for j in range(NP + LAG_P):
        if j + 1 < NP:
            ops.append(("qk", j + 1))
        if j < NP:
            ops.append(("s", j))
        if 0 <= j - LAG_V < NP:
            ops.append(("v", j - LAG_V))
        if j - LAG_V == NP - 1:
            ops.append(("h",))
        if j - LAG_P == NP - NG:
            ops += [("o", 0, G0), ("gate", *range(NP - NG, NP)), ("o", G0, G1)]
        if j - LAG_P >= 0:
            ops.append(("pv", j - LAG_P))
    return ops + [("o", G1, NP)]


def _dot(a, b):
    return jax.lax.dot_general(a, b, (((1,), (0,)), ((), ())), preferred_element_type=F32)


def _dot_nt(a, b):
    return jax.lax.dot_general(a, b, (((1,), (1,)), ((), ())), preferred_element_type=F32)


def _ln(x):
    m = jnp.mean(x, axis=-1, keepdims=True)
    xc = x - m
    v = jnp.mean(xc * xc, axis=-1, keepdims=True)
    return xc * jax.lax.rsqrt(v + 1e-5)


def _rnd(x):
    return x.astype(BF16).astype(F32)


def _ld(ref, rows):
    return jnp.concatenate([ref[t, rows, :] for t in range(ref.shape[0])], axis=1)


def _st(ref, rows, val):
    for t in range(ref.shape[0]):
        ref[t, rows, :] = val[:, t * 128:(t + 1) * 128]


def _kernel(mem0_ref, x_hbm, wq_hbm, wk_hbm, wv_hbm, wo_hbm, *refs):
    late_hbm, out_hbm, late = refs[:NLATE], refs[NLATE], refs[NLATE + 1:2 * NLATE + 1]
    (xin, xout, xpre, hpre, pre, wraw, wqkv, wo32, xs, hz, hbuf, hb16, gate, obuf, bufa, bufb, wpad, wnat,
     sems) = refs[2 * NLATE + 1:]
    wr_ref, wi_ref, g0_ref, g0t_ref, g_ref, gt_ref, m1_ref, m1t_ref, m2_ref, m2t_ref, cf_ref = late

    chunk = lambda n: wraw.at[pl.ds(n * 65, 64), pl.ds(0, 2 * NP)]
    pairs = [(x_hbm.at[pl.ds(0, NPRE), pl.ds(SEG - 8, 8)], xpre),
             (x_hbm.at[pl.ds(0, XHEAD)], xin.at[pl.ds(0, XHEAD)])]
    pairs += [(w.bitcast(U32).at[pl.ds(c * 64, 64)], chunk(3 * c + i))
              for c in range(WCH) for i, w in enumerate((wq_hbm, wk_hbm, wv_hbm))]
    tail = pl.ds(XHEAD, NSEG - XHEAD)
    pairs += [(wo_hbm.bitcast(U32), wo32), (x_hbm.at[tail], xin.at[tail])] + list(zip(late_hbm, late))
    loads = [pltpu.make_async_copy(a, b, sems.at[n]) for n, (a, b) in enumerate(pairs)]
    xp_cp, x_cp, wo_cp = loads[0], loads[1], loads[2 + 3 * WCH]
    xt_cp, late_cp = loads[3 + 3 * WCH], loads[4 + 3 * WCH:]
    out_cp = [pltpu.make_async_copy(xout.at[i], out_hbm.at[:, i], sems.at[len(loads) + i])
              for i in range(N2 // UN)]
    for cp in [xp_cp, *loads[2:2 + 3 * WCH], x_cp, wo_cp]:
        cp.start()

    def filter_prep(c, z):
        for i, w in enumerate((wr_ref, wi_ref)):
            wpad[i, pl.ds(DF - 1, 8), :] = jnp.zeros((8, 128), F32)
            wpad[i, pl.ds(0, DF), :] = w[:, pl.ds(pl.multiple_of(c * 128, 128), 128)].astype(F32)
            wpad[i, pl.ds(DF + 7, 8), :] = obuf[0:8, H * DH - 128:]
            res = lambda r: wpad[i, pl.ds(r + z, 64, stride=5), :]
            top = jnp.concatenate([wpad[i, pl.ds(DF - 1, 8), :], jnp.zeros((56, 128), F32)], axis=0)
            for t, (lo, hi) in enumerate(((res(0), top), (res(1), res(4)), (res(2), res(3)))):
                blk = jnp.concatenate([lo, hi], axis=0).T * cf_ref[:, t * 128:(t + 1) * 128]
                wnat[i, t, pl.ds(2 * c * PA, N1), :] = blk[:N1]
                wnat[i, t, pl.ds((2 * c + 1) * PA, N1), :] = blk[N1:]

    xp_cp.wait()
    for n in range(NPRE):
        _st(hpre, pl.ds(n * 8, 8), _ln(xpre[n].astype(F32)))

    wflat = wraw.reshape(wraw.shape[0] * PW, DH)

    def regroup(n, _, init):
        c, i = n // 3, n % 3
        pltpu.make_async_copy(pairs[2][0], chunk(n), sems.at[2 + n]).wait()
        for j in range(NP):
            a = wflat[pl.ds(n * 65 * PW + j, 64, stride=PW), :]
            b = wflat[pl.ds(n * 65 * PW + j + NP, 64, stride=PW), :]
            w = jnp.concatenate([(a & 0xFFFF) | (b << 16),
                                 (a >> 16) | (b & np.uint32(0xFFFF0000))], axis=1)
            wqkv[j, i, pl.ds(pl.multiple_of(c * 64, 64), 64), :] = w
            t = _dot(hpre[c], pltpu.bitcast(w, BF16))
            pre[j, i] = t if init else pre[j, i] + t
    jax.lax.fori_loop(0, 3, functools.partial(regroup, init=True), None)
    jax.lax.fori_loop(3, 3 * WCH, functools.partial(regroup, init=False), None)
    x_cp.wait()

    ri = jax.lax.broadcasted_iota(jnp.int32, (2 * L, 2 * L), 0)
    ci = jax.lax.broadcasted_iota(jnp.int32, (2 * L, 2 * L), 1)
    same = (ri < L) == (ci < L)
    rl = jnp.where(ri < L, ri, ri - L)
    cl = jnp.where(ci < L, ci, ci - L)
    keep = same & ((rl < M) | (rl >= cl))
    fill = jnp.where(same, -1e9 * LOG2E, -jnp.inf).astype(F32)

    def fetch(l, s):
        r = pl.ds(s * PX, SEG)
        x = xin[jnp.minimum(s, NSEG - 1)].astype(F32)
        if not isinstance(l, int):
            x = jnp.where(l == 0, x, _ld(xs, r))
        _st(xs, r, x)
        h = _ln(x)
        hbuf[0:8, :] = h[SEG - 8:]
        hbuf[8:SEG, :] = h[:SEG - 8]

    def norm(s):
        r = pl.ds(s * PX, SEG)
        _st(hz, r, _ln(_ld(xs, r)))

    def seg(l, s, early=False, first=False):
        r = pl.ds(s * PX, SEG)
        if not first:
            norm(jnp.maximum(s - 1, 0))
        st = {}
        if early:
            hb16[...] = pltpu.bitcast(hbuf[8:L, :].astype(BF16), U32)

        def stack(a, o):
            return jnp.concatenate([a[:, o:o + 128], a[:, o + 128:o + 256]], axis=0)

        def proj(j, parts):
            w = pltpu.bitcast(jnp.concatenate([wqkv[j, i] for i in parts], axis=1), BF16)
            if early:
                a = _dot(pltpu.bitcast(hb16[...], BF16), w)
                last = jnp.concatenate(
                    [pre[j, i, pl.ds(pl.multiple_of(s * 8, 8), 8), :] for i in parts], axis=1)
            else:
                a = _dot(hbuf[...], w)
                last, a = a[:8], a[8:]
            return jnp.concatenate([a[SEG - 8:], a[:SEG - 8], last], axis=0)

        def proj_qk(j):
            a = proj(j, (0, 1))
            st["q", j], st["k", j] = stack(a, 0), stack(a, 256).astype(BF16)

        def proj_v(j):
            st["v", j] = stack(proj(j, (2,)), 0).astype(BF16)

        def scores(j):
            t = _dot_nt(st.pop(("q", j)), st.pop(("k", j))) * (DH ** -0.5 * LOG2E)
            t = jnp.where(keep, t, fill)
            e = jnp.exp2(t - jnp.max(t, axis=-1, keepdims=True))
            st["p", j] = e / jnp.sum(e, axis=-1, keepdims=True)

        def pv(j):
            o = _dot(st.pop(("p", j)), st.pop(("v", j)))
            obuf[:, j * 256:j * 256 + 128] = o[:L]
            obuf[:, j * 256 + 128:(j + 1) * 256] = o[L:]

        def proj_o(a, b):
            return _dot(obuf[:, a * 256:b * 256], pltpu.bitcast(wo32[a * 128:b * 128, :], BF16))

        y = None
        for op, *arg in _schedule():
            if op == "o":
                if first and y is None:
                    wo_cp.wait()
                    for cp in loads[3 + 3 * WCH:]:
                        cp.start()
                y = proj_o(*arg) if y is None else y + proj_o(*arg)
            elif op == "gate":
                if first:
                    continue
                z = (s // NSEG) * 8
                for n, j in enumerate(arg):
                    gate[n, 0:2 * L, 0:2 * L] = st.pop(("p", j))
                _st(gate, pl.ds(2 * L, 8), y[:8])
                for n, j in enumerate(arg):
                    st["p", j] = gate[n, pl.ds(z, 2 * L), 0:2 * L]
            elif op == "h":
                fetch(l, s + 1)
            else:
                {"qk": proj_qk, "v": proj_v, "s": scores, "pv": pv}[op](*arg)
        _st(xs, r, _rnd(_ld(xs, r) + y[M:]))
        hbuf[SEG:L, :] = y[:M]

    def start(l):
        hbuf[SEG:L, :] = mem0_ref[...].astype(F32)
        fetch(l, 0)

    def early_segs(i, _):
        pl.when(i == 1)(xt_cp.wait)
        for u in range(UPRE):
            seg(0, i * UPRE + u + 1, early=True)
    start(0)
    seg(0, 0, early=True, first=True)
    jax.lax.fori_loop(0, (NPRE - 1) // UPRE, early_segs, None)
    for cp in late_cp:
        cp.wait()
    for i in range(NSEG // USEG - S // 128, NPRE // USEG):
        filter_prep(i % (S // 128), 0)

    def layer(l, carry):
        pl.when(l == 1)(lambda: start(l))

        def segs(i, _):
            for u in range(USEG):
                seg(l, i * USEG + u)
            filter_prep(i % (S // 128), i // NSEG)
        jax.lax.fori_loop((1 - l) * (NPRE // USEG), NSEG // USEG, segs, None)
        norm(NSEG - 1)

        def skew(n, first, second):
            prev = first(0)
            for u in range(n):
                nxt = first(u + 1) if u + 1 < n else None
                second(u, prev)
                prev = nxt

        tile = lambda a, t: a[:, t * 128:(t + 1) * 128]

        def fwd(i, _):
            def feat(u):
                r = pl.ds(i * UN + u, N1, stride=PX)
                z0, z1, z2, z3, z4 = (hz[t, r, :] for t in range(NT))
                s1, d1, s2, d2 = z1 + z4, z1 - z4, z2 + z3, z2 - z3
                u1 = jnp.concatenate([z0 + C1 * s1 + C2 * s2, -S1 * d1 - S2 * d2], axis=1)
                u2 = jnp.concatenate([z0 + C2 * s1 + C1 * s2, S1 * d2 - S2 * d1], axis=1)
                xf = [_dot(z0 + s1 + s2, g0_ref[...]), _dot(u1, g_ref[0]), _dot(u2, g_ref[1])]
                return jnp.concatenate(
                    [jnp.concatenate([tile(a, c) for a in xf], axis=1) for c in range(2)],
                    axis=0).astype(BF16)

            def seq(u, zf):
                n2 = i * UN + u
                a = _dot(m1_ref[n2], zf)
                _st(bufa, pl.ds(n2, N1, stride=PA), a[:N1])
                _st(bufa, pl.ds(n2 + N2, N1, stride=PA), a[N1:])
            skew(UN, feat, seq)
        jax.lax.fori_loop(0, N2 // UN, fwd, None)

        def mid(i, _):
            rows = lambda u, w: pl.ds((2 * (i * UN + u) + w) * PA, 2 * N2)

            def f2(u):
                a = jnp.concatenate([_ld(bufa, rows(u, 0)), _ld(bufa, rows(u, 1))], axis=0)
                xf = _dot(m2_ref[...], a.astype(BF16))
                ys = []
                for w in range(2):
                    kr = pl.ds(2 * (i * UN + u) + w, N2, stride=PA)
                    wr, wi = _ld(wnat.at[0], kr), _ld(wnat.at[1], kr)
                    xr, xi = xf[w * 64:w * 64 + 32], xf[w * 64 + 32:w * 64 + 64]
                    ys += [xr * wr - xi * wi, xr * wi + xi * wr]
                return jnp.concatenate(ys, axis=0).astype(BF16)

            def i2(u, y):
                b = _dot(m2t_ref[...], y)
                _st(bufb, rows(u, 0), b[:64])
                _st(bufb, rows(u, 1), b[64:])
            skew(UN, f2, i2)
        jax.lax.fori_loop(0, N1 // 2 // UN, mid, None)

        def inv(i, _):
            def seq(u):
                n2 = i * UN + u
                b = jnp.concatenate([_ld(bufb, pl.ds(n2, N1, stride=PA)),
                                     _ld(bufb, pl.ds(n2 + N2, N1, stride=PA))], axis=0)
                return _dot(m1t_ref[n2], b.astype(BF16)).astype(BF16)

            def feat(u, yf):
                ri_ = lambda t: jnp.concatenate([tile(yf[:N1], t), tile(yf[N1:], t)], axis=1)
                v0 = _dot(ri_(0), g0t_ref[...])
                v1, v2 = _dot(ri_(1), gt_ref[0]), _dot(ri_(2), gt_ref[1])
                a1, b1, a2, b2 = tile(v1, 0), tile(v1, 1), tile(v2, 0), tile(v2, 1)
                s1, s2 = v0 + C1 * a1 + C2 * a2, v0 + C2 * a1 + C1 * a2
                d1, d2 = -S1 * b1 - S2 * b2, S1 * b2 - S2 * b1
                y = jnp.concatenate([v0 + a1 + a2, s1 + d1, s2 + d2, s2 - d2, s1 - d1], axis=1)
                r = pl.ds(i * UN + u, N1, stride=PX)
                _st(xs, r, _rnd(_ld(xs, r) + y))
            skew(UN, seq, feat)

            for c, cp in enumerate(out_cp):
                @pl.when(l * len(out_cp) + i == len(out_cp) + c)
                def _():
                    for n1 in range(N1):
                        xout[c, n1] = _ld(xs, pl.ds(n1 * PX + c * UN, UN)).astype(BF16)
                    cp.start()
        jax.lax.fori_loop(0, N2 // UN, inv, None)
        return carry
    jax.lax.fori_loop(0, 2, layer, 0)

    for cp in out_cp:
        cp.wait()


@functools.partial(jax.jit, static_argnames=("A_seg_len",))
def pallas_interleave_layers__memory_aug_recurrent_mem_tr__spectral_gfnet__prompt_kernel(
    A_x, A_mem0, A_Wq, A_Wk, A_Wv, A_Wo, A_seg_len, B_x, B_w_r, B_w_i,
):
    del B_x
    assert A_seg_len == SEG and A_x.shape == (1, S, D) and A_Wq.shape == (D, H, DH)
    vmem = pl.BlockSpec(memory_space=pltpu.VMEM)
    hbm = pl.BlockSpec(memory_space=pl.ANY)
    late = (B_w_r.T, B_w_i.T, *_consts())
    assert len(late) == NLATE
    out = pl.pallas_call(
        _kernel,
        out_shape=jax.ShapeDtypeStruct((N1, N2 // UN, UN, D), BF16),
        in_specs=[vmem] + [hbm] * (5 + NLATE),
        out_specs=hbm,
        scratch_shapes=[pltpu.VMEM(a.shape, a.dtype) for a in late] + [
            pltpu.VMEM((NSEG, SEG, D), BF16),
            pltpu.VMEM((N2 // UN, N1, UN, D), BF16),
            pltpu.VMEM((NPRE, 8, D), BF16),
            pltpu.VMEM((NT, NPRE * 8, 128), F32),
            pltpu.VMEM((NP, 3, NPRE * 8, 256), F32),
            pltpu.VMEM((3 * WCH * 65, PW, DH), U32),
            pltpu.VMEM((NP, 3, D // 2, 256), U32),
            pltpu.VMEM((H * DH // 2, D), U32),
            pltpu.VMEM((NT, (NSEG + 2) * PX, 128), F32),
            pltpu.VMEM((NT, (NSEG + 2) * PX, 128), F32),
            pltpu.VMEM((L, D), F32),
            pltpu.VMEM((SEG // 2, D), U32),
            pltpu.VMEM((NT, 2 * L + 16, 128), F32),
            pltpu.VMEM((L, H * DH), F32),
            pltpu.VMEM((NF, (N1 + 2) * PA, 128), F32),
            pltpu.VMEM((NF, (N1 + 2) * PA, 128), F32),
            pltpu.VMEM((2, DF + 15, 128), F32),
            pltpu.VMEM((2, NF, (N2 + 2) * PA, 128), F32),
            pltpu.SemaphoreType.DMA((3 * WCH + 4 + NLATE + N2 // UN,)),
        ],
        compiler_params=pltpu.CompilerParams(vmem_limit_bytes=120 * 1024 * 1024),
    )(A_mem0.reshape(M, D), A_x.reshape(NSEG, SEG, D),
      A_Wq.reshape(D // 2, 2 * H, DH), A_Wk.reshape(D // 2, 2 * H, DH), A_Wv.reshape(D // 2, 2 * H, DH),
      A_Wo.reshape(H * DH, D), *late)
    return out.reshape(1, S, D)
```
